```python
import jax
import jax.numpy as jnp

def _softmax(x, axis=-1):
    return jax.nn.softmax(x, axis=axis)
def _gelu(x):
    return jax.nn.gelu(x, approximate=True)
def _silu(x):
    return jax.nn.silu(x)
def _sigmoid(x):
    return jax.nn.sigmoid(x)
def _layernorm(x, axis=-1, eps=1e-5):
    m = jnp.mean(x, axis=axis, keepdims=True)
    v = jnp.var(x, axis=axis, keepdims=True)
    return (x - m) / jnp.sqrt(v + eps)
def _scatter_add(tgt, idx, src, axis=0):
    return tgt.at[idx].add(src)
def _segment_sum(src, seg, n):
    return jax.ops.segment_sum(src, seg, n)
class _Rng:
    def __init__(self, key):
        self._k = key
    def _next(self):
        self._k, sub = jax.random.split(self._k)
        return sub
    def normal(self, shape):
        return jax.random.normal(self._next(), shape, dtype=jnp.bfloat16)
    def randint(self, lo, hi, shape):
        return jax.random.randint(self._next(), shape, lo, hi, dtype=jnp.int32)
    def uniform(self, shape, lo=0.0, hi=1.0):
        return jax.random.uniform(self._next(), shape, jnp.bfloat16, lo, hi)
    def permutation(self, n):
        return jax.random.permutation(self._next(), n)


kernel_name = 'standalone__fused_io_aware_attn__prompt'

def setup_inputs():
    _rng = _Rng(jax.random.key(int.from_bytes(__import__("os").urandom(4), "little")))
    _w = (lambda a: (lambda t: t.astype(jnp.bfloat16) if jnp.issubdtype(t.dtype, jnp.floating) else t)(jnp.asarray(a)))
    B, H, S = 2, 32, 2048
    Dh = max(1, 1024 // 32)
    return {
        "q": _w((lambda *s: _rng.normal(s) * 0.05)(B, H, S, Dh)),
        "k": _w((lambda *s: _rng.normal(s) * 0.05)(B, H, S, Dh)),
        "v": _w((lambda *s: _rng.normal(s) * 0.05)(B, H, S, Dh)),
    }

def reference(q, k, v):
    scale = q.shape[-1] ** -0.5
    s = jnp.einsum('bhqd,bhkd->bhqk', q, k) * scale
    p = _softmax(s, axis=-1)
    return jnp.einsum('bhqk,bhkd->bhqd', p, v)
```

```python
import jax
import jax.numpy as jnp
from jax import lax
import jax.experimental.pallas as pl
import jax.experimental.pallas.tpu as pltpu

_LOG2E = 1.4426950408889634
_T = 128
_KA = 80
_HB = 4
_LAG = 6
_START = 32
_KCH = 256
_BMAX = 8.0
_TS = 512

_f32, _bf16, _i32, _u32 = jnp.float32, jnp.bfloat16, jnp.int32, jnp.uint32


def _kernel(q_ref, k_ref, v_ref, qn_ref, kn_ref, vn_ref, o_ref,
            ka_scr, vf_scr, o0_scr, st_scr, ks_scr):
    T, HB = _T, _HB
    _, D, S = k_ref.shape
    NC = S // T
    NQ = S // (2 * T)
    c0 = D ** -0.5 * _LOG2E

    def rev(x):
        return jnp.concatenate(
            [x[g * 8:g * 8 + 8] for g in reversed(range(T // 8))], axis=0)

    def refs(h):
        if h < HB:
            return q_ref.at[h], k_ref.at[h], v_ref.at[h]
        return qn_ref.at[0], kn_ref.at[0], vn_ref.at[0]

    def run(units, kmaxs, out, kch):
        accs, ls, ps, ws = {}, {}, {}, {}

        def prep_kmax(h):
            _, kr, vr = refs(h)
            m = None
            for c in range(S // kch):
                kf = kr[:, c * kch:(c + 1) * kch].astype(_f32)
                vw = pltpu.bitcast(vr[:, c * kch:(c + 1) * kch], _i32)
                vb = vw[0:8] | vw[8:16]
                vb = pltpu.bitcast((vb | (vb << 16)) & 0x60000000, _f32)
                kn = jnp.concatenate(
                    [jnp.sum(kf * kf, axis=0, keepdims=True),
                     jnp.max(vb, axis=0, keepdims=True)], axis=0)
                if m is not None:
                    kn = jnp.maximum(kn, m)
                m = jnp.max(kn, axis=1, keepdims=True)
            mb = jnp.broadcast_to(m, (2, T))
            kmaxs[h] = jnp.where(mb[1:2] == 0.0, jnp.inf, mb[0:1] * 1.05)

        def prep_w(h, i):
            qs = refs(h)[0][:, 2 * i * T:(2 * i + 2) * T].astype(_f32) * c0
            qn = jnp.sum(qs * qs, axis=0, keepdims=True)
            b2 = jnp.maximum(qn[:, :T], qn[:, T:]) * kmaxs[h]
            b2 = jnp.maximum(b2, 2.0 ** -40)
            e2 = (pltpu.bitcast(b2, _i32) >> 23) + 1
            b = pltpu.bitcast(((e2 + 128) >> 1) << 23, _f32)
            b = jnp.where(b2 < _BMAX * _BMAX, b, jnp.nan)
            row = lax.broadcasted_iota(_i32, (16, T), 0)
            coef = jnp.where(
                row == 0, -2.0 ** 24, jnp.where(
                    row == 4, -1.5 * 2.0 ** 12, jnp.where(
                        row == 8, 2.0 ** 24, jnp.where(row == 12, -1.0, 0.0))))
            ws[h, i] = jnp.concatenate(
                [qs[:, :T] * 2.0 ** 11, coef * b, qs[:, T:]], axis=0).astype(_bf16)

        def prep_kv(h, c):
            _, kr, vr = refs(h)
            kc = kr[:, c * T:(c + 1) * T].astype(_f32)
            ka = rev(jnp.concatenate([kc, jnp.ones((16, T), _f32), kc], axis=0).T)
            ka_scr[h % 2, c * T // 2:(c + 1) * T // 2, :] = pltpu.bitcast(
                ka.astype(_bf16), _u32)
            vf_scr[h % 2, :, c * T:(c + 1) * T] = vr[:, c * T:(c + 1) * T].astype(_f32)

        def qk(u):
            h, i, c = u
            if i == 0 and c == 0:
                prep_kmax(h)
            if c == 0:
                prep_w(h, i)
            if i == 0:
                prep_kv(h, c)
            kc = pltpu.bitcast(ka_scr[h % 2, c * T // 2:(c + 1) * T // 2, :], _bf16)
            t = jnp.dot(kc, ws[h, i], preferred_element_type=_f32)
            hi = pltpu.bitcast(pltpu.bitcast(t, _i32) & (-4096), _f32)
            p = jnp.concatenate(
                [jnp.exp2(t * 2.0 ** -11), jnp.exp2(t - hi)], axis=1)
            part = jnp.sum(p.reshape(T // 8, 8, 2 * T), axis=0)
            ls[h, i] = part if c == 0 else ls[h, i] + part
            ps[u] = rev(p)

        def pv(u):
            h, i, c = u
            r = jnp.dot(vf_scr[h % 2, :, c * T:(c + 1) * T], ps.pop(u),
                        preferred_element_type=_f32)
            accs[h, i] = r if c == 0 else accs[h, i] + r
            if c == NC - 1:
                lsum = jnp.sum(ls[h, i], axis=0, keepdims=True)
                val = (accs[h, i] * pl.reciprocal(lsum, approx=False)).astype(o_ref.dtype)
                out(h, i, val, lsum[:, :T])

        for j in range(len(units) + _LAG):
            if j < len(units):
                qk(units[j])
            if j >= _LAG:
                pv(units[j - _LAG])

    @pl.when(pl.program_id(0) == 0)
    def _():
        kmaxs0 = {}

        def out0(h, i, val, lsum):
            o0_scr[...] = val
            st_scr[1:2, :] = lsum

        run([(0, 0, c) for c in range(NC)], kmaxs0, out0, S)
        st_scr[0:1, :] = kmaxs0[0]

    kmaxs = {0: st_scr[0:1, :]}
    chk = [st_scr[1:2, :]]
    o_ref[0, :, 0:2 * T] = o0_scr[...]
    units = []
    for h in range(HB):
        rest = [(h, i, c) for i in range(1, NQ) for c in range(NC)]
        n = len(rest) - _START
        pos = [_START + (c * n) // NC for c in range(NC)]
        for j, u in enumerate(rest):
            if j in pos:
                units.append((h + 1, 0, pos.index(j)))
            units.append(u)

    def out(h, i, val, lsum):
        if h < HB:
            o_ref[h, :, 2 * i * T:2 * (i + 1) * T] = val
            chk[0] = chk[0] + lsum
        else:
            o0_scr[...] = val
            st_scr[1:2, :] = lsum
            st_scr[0:1, :] = jnp.maximum(kmaxs[HB], -lsum)

    run(units, kmaxs, out, _KCH)
    total = jnp.sum(chk[0])

    @pl.when(jnp.logical_not(total < 1e30))
    def _():
        def head(h, carry):
            ks_scr[...] = k_ref[h].astype(_f32).T.astype(_bf16)

            def tile(j, carry):
                off = pl.multiple_of(j * _TS, _TS)
                s = jnp.dot(ks_scr[...], q_ref[h, :, pl.ds(off, _TS)],
                            preferred_element_type=_f32)
                m = jnp.max(s, axis=0, keepdims=True)
                p = jnp.exp2((s - m) * c0)
                l = jnp.sum(p, axis=0, keepdims=True)
                o = jnp.dot(v_ref[h], p.astype(_bf16), preferred_element_type=_f32)
                o_ref[h, :, pl.ds(off, _TS)] = (o / l).astype(o_ref.dtype)
                return carry

            return lax.fori_loop(0, S // _TS, tile, carry)

        lax.fori_loop(0, HB, head, 0)


@jax.jit
def pallas_standalone__fused_io_aware_attn__prompt_kernel(
    q: jax.Array,
    k: jax.Array,
    v: jax.Array,
):
    B, H, S, D = q.shape
    BH = B * H
    HB, T = _HB, _T
    qt, kt, vt = (jnp.swapaxes(x, -1, -2).reshape(BH, D, S) for x in (q, k, v))
    spec = pl.BlockSpec((HB, D, S), lambda s: (s, 0, 0))

    def nxt(s):
        return (jnp.minimum((s + 1) * HB, BH - 1), 0, 0)

    o = pl.pallas_call(
        _kernel,
        grid=(BH // HB,),
        in_specs=[spec, spec, spec,
                  pl.BlockSpec((1, D, 2 * T), nxt),
                  pl.BlockSpec((1, D, S), nxt),
                  pl.BlockSpec((1, D, S), nxt)],
        out_specs=spec,
        out_shape=jax.ShapeDtypeStruct((BH, D, S), q.dtype),
        scratch_shapes=[
            pltpu.VMEM((2, S // 2, _KA), _u32),
            pltpu.VMEM((2, D, S), _f32),
            pltpu.VMEM((D, 2 * T), q.dtype),
            pltpu.VMEM((8, T), _f32),
            pltpu.VMEM((S, D), _bf16),
        ],
        compiler_params=pltpu.CompilerParams(
            dimension_semantics=("arbitrary",),
            vmem_limit_bytes=100 * 1024 * 1024),
    )(qt, kt, vt, qt, kt, vt)
    return jnp.swapaxes(o.reshape(B, H, D, S), -1, -2)
```

```python
import jax
import jax.numpy as jnp
from jax import lax
import jax.experimental.pallas as pl
import jax.experimental.pallas.tpu as pltpu

_LOG2E = 1.4426950408889634
_T = 128
_KA = 80
_HB = 7
_LAG = 6
_ENDL = 3
_START = 52
_KCH = 256
_BMAX = 8.0
_TINY = 2.0 ** -110
_TS = 512

_f32, _bf16, _i32, _u32 = jnp.float32, jnp.bfloat16, jnp.int32, jnp.uint32


def _kernel(q_hbm, k_hbm, v_hbm, o_hbm, q_all, k_all, v_all, o_all,
            ka_scr, vf_scr, st_scr, fl_scr, ks_scr, isem, osem):
    T, HB = _T, _HB
    BH, D, S = q_hbm.shape
    NS = (BH - 1) // HB
    NC = S // T
    NQ = S // (2 * T)
    c0 = D ** -0.5 * _LOG2E

    def in_copies(g, n, slot):
        return [pltpu.make_async_copy(a.at[pl.ds(g, n)], b.at[pl.ds(g, n)], isem.at[slot])
                for a, b in ((k_hbm, k_all), (v_hbm, v_all), (q_hbm, q_all))]

    def out_copy(g, lo, hi):
        return pltpu.make_async_copy(o_all.at[g, :, pl.ds(lo, hi - lo)],
                                     o_hbm.at[g, :, pl.ds(lo, hi - lo)], osem.at[0])

    def prep_kmax(g, kch):
        m = None
        for c in range(S // kch):
            kf = k_all[g, :, c * kch:(c + 1) * kch].astype(_f32)
            vw = pltpu.bitcast(v_all[g, :, c * kch:(c + 1) * kch], _i32)
            vb = vw[0:8] | vw[8:16]
            vb = pltpu.bitcast((vb | (vb << 16)) & 0x60000000, _f32)
            kn = jnp.concatenate(
                [jnp.sum(kf * kf, axis=0, keepdims=True),
                 jnp.max(vb, axis=0, keepdims=True)], axis=0)
            if m is not None:
                kn = jnp.maximum(kn, m)
            m = jnp.max(kn, axis=1, keepdims=True)
        mb = jnp.broadcast_to(m, (2, T))
        return jnp.where(mb[1:2] == 0.0, jnp.inf, jnp.maximum(mb[0:1], _TINY) * 1.05)

    def prep_w(g, i, kmax):
        qs = q_all[g, :, 2 * i * T:(2 * i + 2) * T].astype(_f32) * c0
        qn = jnp.sum(qs * qs, axis=0, keepdims=True)
        qn = jnp.maximum(jnp.maximum(qn[:, :T], qn[:, T:]), _TINY)
        b2 = jnp.maximum(qn * kmax, 2.0 ** -40)
        e2 = (pltpu.bitcast(b2, _i32) >> 23) + 1
        b = pltpu.bitcast(((e2 + 128) >> 1) << 23, _f32)
        b = jnp.where(b2 < _BMAX * _BMAX, b, jnp.nan)
        row = lax.broadcasted_iota(_i32, (16, T), 0)
        coef = jnp.where(
            row == 0, -2.0 ** 24, jnp.where(
                row == 4, -1.5 * 2.0 ** 12, jnp.where(
                    row == 8, 2.0 ** 24, jnp.where(row == 12, -1.0, 0.0))))
        return jnp.concatenate(
            [qs[:, :T] * 2.0 ** 11, coef * b, qs[:, T:]], axis=0).astype(_bf16)

    def prep_kv(g, buf, c):
        kc = k_all[g, :, c * T:(c + 1) * T]
        ka = jnp.concatenate([kc, jnp.ones((16, T), _bf16), kc], axis=0).T
        kw = pltpu.bitcast(ka, _u32)
        ka_scr[buf, c * T // 2:(c + 1) * T // 2, :] = jnp.concatenate(
            [pltpu.roll(kw[j * 8:j * 8 + 8], 4, 0) for j in reversed(range(T // 16))],
            axis=0)
        vf_scr[buf, :, c * T:(c + 1) * T] = v_all[g, :, c * T:(c + 1) * T].astype(_f32)

    def rev(x):
        return jnp.concatenate(
            [x[j * 8:j * 8 + 8] for j in reversed(range(T // 8))], axis=0)

    def block(gs, bufs):
        nh = len(gs) - 1
        units = []
        for h in range(nh):
            rest = [(h, i, c) for i in range(1, NQ) for c in range(NC)]
            n = len(rest) - _START
            pos = [_START + (c * n) // NC for c in range(NC)]
            for j, u in enumerate(rest):
                if j in pos:
                    units.append((h + 1, 0, pos.index(j)))
                units.append(u)
        accs, ls, ps, ws, chk = {}, {}, {}, {}, {}
        kmaxs = {0: st_scr[0:1, :]}

        def qk(u):
            h, i, c = u
            g, buf = gs[h], bufs[h]
            if i == 0 and c == 0:
                kmaxs[h] = prep_kmax(g, _KCH)
            if c == 0:
                ws[h, i] = prep_w(g, i, kmaxs[h])
            if i == 0:
                prep_kv(g, buf, c)
            kc = pltpu.bitcast(ka_scr[buf, c * T // 2:(c + 1) * T // 2, :], _bf16)
            t = jnp.dot(kc, ws[h, i], preferred_element_type=_f32)
            hi = pltpu.bitcast(pltpu.bitcast(t, _i32) & (-4096), _f32)
            p = jnp.concatenate(
                [jnp.exp2(t * 2.0 ** -11), jnp.exp2(t - hi)], axis=1)
            part = jnp.sum(p.reshape(T // 8, 8, 2 * T), axis=0)
            ls[h, i] = part if c == 0 else ls[h, i] + part
            if h < nh and i < NQ - 1 and c == (12 if i == 0 else 4):
                kmaxs[h] = jnp.maximum(kmaxs[h], -part[0:1, :T])
            ps[u] = rev(p)

        def pv(u):
            h, i, c = u
            g, buf = gs[h], bufs[h]
            r = jnp.dot(vf_scr[buf, :, c * T:(c + 1) * T], ps.pop(u),
                        preferred_element_type=_f32)
            accs[h, i] = r if c == 0 else accs[h, i] + r
            if c < NC - 1:
                return
            lsum = jnp.sum(ls[h, i], axis=0, keepdims=True)
            o_all[g, :, 2 * i * T:2 * (i + 1) * T] = (
                accs[h, i] * pl.reciprocal(lsum, approx=False)).astype(o_all.dtype)
            l1 = lsum[:, :T]
            if i == 0:
                fl_scr[0, pl.ds(g, 1), :] = l1
                if h == nh:
                    st_scr[0:1, :] = jnp.maximum(kmaxs[h], -l1)
                    out_copy(g, 0, 2 * T).start()
            else:
                chk[h] = l1 if i == 1 else chk[h] + l1
                if i == NQ - 1:
                    fl_scr[1, pl.ds(g, 1), :] = chk[h]
                    out_copy(g, 2 * T if h == 0 else 0, S).start()

        done = 0
        for j in range(len(units)):
            qk(units[j])
            if _LAG <= j < len(units) - _ENDL:
                pv(units[done])
                done += 1
        while done < len(units):
            pv(units[done])
            done += 1

    bufs = [h % 2 for h in range(HB)] + [0]
    if HB % 2:
        bufs[HB - 1] = 2

    for g, n, slot in ((0, 1, 0), (1, 1, 1), (2, HB, 2)):
        for cp in in_copies(g, n, slot):
            cp.start()
    for cp in in_copies(0, 1, 0):
        cp.wait()
    st_scr[0:1, :] = prep_kmax(0, S)
    for c in range(NC):
        prep_kv(0, 1, c)
    for cp in in_copies(1, 1, 1):
        cp.wait()
    block([0, 1], [1, 0])

    def step(s, carry):
        base = 1 + s * HB

        @pl.when(s < NS - 1)
        def _():
            for cp in in_copies(base + 1, HB, 2):
                cp.wait()

        @pl.when(s == NS - 1)
        def _():
            for cp in in_copies(base + 1, HB - 1, 2):
                cp.wait()

        @pl.when(s < NS - 2)
        def _():
            for cp in in_copies(base + 1 + HB, HB, 2):
                cp.start()

        @pl.when(s == NS - 2)
        def _():
            for cp in in_copies(base + 1 + HB, HB - 1, 2):
                cp.start()

        nxt = jnp.where(s == NS - 1, 0, base + HB)
        block([base + h for h in range(HB)] + [nxt], bufs)
        return carry

    lax.fori_loop(0, NS, step, 0)

    total = jnp.sum(fl_scr[0] + fl_scr[1])
    pltpu.make_async_copy(o_all, o_hbm, osem.at[0]).wait()

    @pl.when(jnp.logical_not(total < 1e30))
    def _():
        def head(g, carry):
            tg = jnp.sum(fl_scr[0, pl.ds(g, 1), :] + fl_scr[1, pl.ds(g, 1), :])

            @pl.when(jnp.logical_not(tg < 1e30))
            def _():
                ks_scr[...] = k_all[g].astype(_f32).T.astype(_bf16)

                def tile(j, carry):
                    off = pl.multiple_of(j * _TS, _TS)
                    s = jnp.dot(ks_scr[...], q_all[g, :, pl.ds(off, _TS)],
                                preferred_element_type=_f32)
                    m = jnp.max(s, axis=0, keepdims=True)
                    p = jnp.exp2((s - m) * c0)
                    l = jnp.sum(p, axis=0, keepdims=True)
                    o = jnp.dot(v_all[g], p.astype(_bf16), preferred_element_type=_f32)
                    o_all[g, :, pl.ds(off, _TS)] = (o / l).astype(o_all.dtype)
                    return carry

                lax.fori_loop(0, S // _TS, tile, 0)
                cp = out_copy(g, 0, S)
                cp.start()
                cp.wait()

            return carry

        lax.fori_loop(0, BH, head, 0)


@jax.jit
def pallas_standalone__fused_io_aware_attn__prompt_kernel(
    q: jax.Array,
    k: jax.Array,
    v: jax.Array,
):
    B, H, S, D = q.shape
    BH = B * H
    assert (BH - 1) % _HB == 0 and (BH - 1) // _HB >= 2 and D == 32
    qt, kt, vt = (jnp.swapaxes(x, -1, -2).reshape(BH, D, S) for x in (q, k, v))
    hbm = pl.BlockSpec(memory_space=pl.ANY)
    o = pl.pallas_call(
        _kernel,
        in_specs=[hbm, hbm, hbm],
        out_specs=hbm,
        out_shape=jax.ShapeDtypeStruct((BH, D, S), q.dtype),
        scratch_shapes=[
            pltpu.VMEM((BH, D, S), q.dtype),
            pltpu.VMEM((BH, D, S), q.dtype),
            pltpu.VMEM((BH, D, S), q.dtype),
            pltpu.VMEM((BH, D, S), q.dtype),
            pltpu.VMEM((3, S // 2, _KA), _u32),
            pltpu.VMEM((3, D, S), _f32),
            pltpu.VMEM((8, _T), _f32),
            pltpu.VMEM((2, BH, _T), _f32),
            pltpu.VMEM((S, D), _bf16),
            pltpu.SemaphoreType.DMA((3,)),
            pltpu.SemaphoreType.DMA((1,)),
        ],
        compiler_params=pltpu.CompilerParams(
            vmem_limit_bytes=100 * 1024 * 1024,
            disable_bounds_checks=True),
    )(qt, kt, vt)
    return jnp.swapaxes(o.reshape(B, H, D, S), -1, -2)
```

```python
import jax
import jax.numpy as jnp
from jax import lax
import jax.experimental.pallas as pl
import jax.experimental.pallas.tpu as pltpu

_LOG2E = 1.4426950408889634
_T = 128
_KA = 80
_HB = 7
_LAG = 6
_ENDL = 5
_START = 76
_KDEP = (12, 7)
_NA = 2
_NPRE = 6
_BMAX = 8.0
_TINY = 2.0 ** -110
_TS = 512

_f32, _bf16, _i32, _u32 = jnp.float32, jnp.bfloat16, jnp.int32, jnp.uint32


@jax.jit
def _stage_k(kc):
    ka = jnp.concatenate([kc, jnp.ones((16, _T), _bf16), kc], axis=0).T
    kw = pltpu.bitcast(ka, _u32)
    return jnp.concatenate(
        [pltpu.roll(kw[j * 8:j * 8 + 8], 4, 0) for j in reversed(range(_T // 16))],
        axis=0)


@jax.jit
def _probs(kw, w):
    t = jnp.dot(pltpu.bitcast(kw, _bf16), w, preferred_element_type=_f32)
    hi = pltpu.bitcast(pltpu.bitcast(t, _i32) & (-4096), _f32)
    p = jnp.concatenate([jnp.exp2(t * 2.0 ** -11), jnp.exp2(t - hi)], axis=1)
    part = jnp.sum(p.reshape(_T // 8, 8, 2 * _T), axis=0)
    p = jnp.concatenate(
        [p[j * 8:j * 8 + 8] for j in reversed(range(_T // 8))], axis=0)
    return p, part


@jax.jit
def _norms(kc, vc):
    kf = kc.astype(_f32)
    vw = pltpu.bitcast(vc, _i32)
    vb = vw[0:8] | vw[8:16]
    vb = pltpu.bitcast((vb | (vb << 16)) & 0x60000000, _f32)
    return jnp.concatenate(
        [jnp.sum(kf * kf, axis=0, keepdims=True),
         jnp.max(vb, axis=0, keepdims=True)], axis=0)


@jax.jit
def _weights(q, kmax):
    qs = q.astype(_f32) * (q.shape[0] ** -0.5 * _LOG2E)
    qn = jnp.sum(qs * qs, axis=0, keepdims=True)
    qn = jnp.maximum(jnp.maximum(qn[:, :_T], qn[:, _T:]), _TINY)
    b2 = jnp.maximum(qn * kmax, 2.0 ** -40)
    e2 = (pltpu.bitcast(b2, _i32) >> 23) + 1
    b = pltpu.bitcast(((e2 + 128) >> 1) << 23, _f32)
    b = jnp.where(b2 < _BMAX * _BMAX, b, jnp.nan)
    row = lax.broadcasted_iota(_i32, (16, _T), 0)
    coef = jnp.where(
        row == 0, -2.0 ** 24, jnp.where(
            row == 4, -1.5 * 2.0 ** 12, jnp.where(
                row == 8, 2.0 ** 24, jnp.where(row == 12, -1.0, 0.0))))
    return jnp.concatenate(
        [qs[:, :_T] * 2.0 ** 11, coef * b, qs[:, _T:]], axis=0).astype(_bf16)


def _kernel(q_hbm, k_hbm, v_hbm, o_hbm, q_all, k_all, v_all, o_all,
            ka_scr, vf_scr, st_scr, w_scr, fl_scr, ks_scr, isem, osem):
    T, HB = _T, _HB
    BH, D, S = q_hbm.shape
    NS = (BH - 1) // HB
    NC = S // T
    NQ = S // (2 * T)

    def in_copies(g, n, slot):
        return [pltpu.make_async_copy(a.at[pl.ds(g, n)], b.at[pl.ds(g, n)], isem.at[slot])
                for a, b in ((k_hbm, k_all), (v_hbm, v_all), (q_hbm, q_all))]

    def cols_copy(src, dst, g, lo, hi, sem):
        return pltpu.make_async_copy(src.at[g, :, pl.ds(lo, hi - lo)],
                                     dst.at[g, :, pl.ds(lo, hi - lo)], sem)

    def out_copy(g, lo, hi):
        return cols_copy(o_all, o_hbm, g, lo, hi, osem.at[0])

    def max_key_norm(g):
        m = None
        for c in range(NC):
            kn = _norms(k_all[g, :, c * T:(c + 1) * T], v_all[g, :, c * T:(c + 1) * T])
            if m is not None:
                kn = jnp.maximum(kn, m)
            m = jnp.max(kn, axis=1, keepdims=True)
        mb = jnp.broadcast_to(m, (2, T))
        return jnp.where(mb[1:2] == 0.0, jnp.inf, jnp.maximum(mb[0:1], _TINY) * 1.05)

    def weights(g, i, kmax):
        return _weights(q_all[g, :, 2 * i * T:(2 * i + 2) * T], kmax)

    def stage_k(g, buf, c):
        ka_scr[buf, c * T // 2:(c + 1) * T // 2, :] = _stage_k(k_all[g, :, c * T:(c + 1) * T])

    def stage_v(g, buf, c):
        vf_scr[buf, :, c * T:(c + 1) * T] = v_all[g, :, c * T:(c + 1) * T].astype(_f32)

    def block(gs, bufs, lo=1, hi=None):
        first = hi is not None
        nh = 1 if first else len(gs) - 1
        units = []
        for h in range(nh):
            rest = [(h, i, c) for i in range(1, NQ) for c in range(NC)]
            n = len(rest) - _START
            pos = [] if first else [_START + (c * n) // NC for c in range(NC)]
            for j, u in enumerate(rest):
                if j in pos:
                    units.append((h + 1, 0, pos.index(j)))
                if h > 0 or lo <= u[1] < (hi or NQ):
                    units.append(u)
        accs, ls, ps, ws, chk = {}, {}, {}, {}, {}
        kmaxs = {0: st_scr[0:1, :]}
        if not first:
            ws[0, lo] = pltpu.bitcast(w_scr[...], _bf16)
        if lo > 1:
            chk[0] = st_scr[1:2, :]

        def qk(u):
            h, i, c = u
            g, buf = gs[h], bufs[h]
            if i == 0 and c == 0:
                kmaxs[h] = max_key_norm(g)
            if (h, i) not in ws:
                ws[h, i] = weights(g, i, kmaxs[h])
            if i == 0 or (first and i == 1):
                if i == 0 or c >= _NPRE:
                    stage_k(g, buf, c)
                stage_v(g, buf, c)
            ps[u], part = _probs(ka_scr[buf, c * T // 2:(c + 1) * T // 2, :], ws[h, i])
            ls[h, i] = part if c == 0 else ls[h, i] + part
            if i < NQ - 1 and c == _KDEP[min(i, 1)]:
                kmaxs[h] = jnp.maximum(kmaxs[h], -part[0:1, :T])
                if h == nh:
                    st_scr[0:1, :] = kmaxs[h]
                if h == nh or (first and i == hi - 1):
                    w_scr[...] = pltpu.bitcast(weights(g, i + 1, kmaxs[h]), _u32)

        def pv(u):
            h, i, c = u
            g, buf = gs[h], bufs[h]
            r = jnp.dot(vf_scr[buf, :, c * T:(c + 1) * T], ps.pop(u),
                        preferred_element_type=_f32)
            accs[h, i] = r if c == 0 else accs[h, i] + r
            if c < NC - 1:
                return
            lsum = jnp.sum(ls[h, i], axis=0, keepdims=True)
            o_all[g, :, 2 * i * T:2 * (i + 1) * T] = (
                accs[h, i] * pl.reciprocal(lsum, approx=False)).astype(o_all.dtype)
            l1 = lsum[:, :T]
            if i == 0:
                fl_scr[0, pl.ds(g, 1), :] = l1
                if h == nh:
                    out_copy(g, 0, 2 * T).start()
                return
            chk[h] = chk[h] + l1 if h in chk else l1
            olo = 2 * T if h == 0 else 0
            if first and i == hi - 1:
                st_scr[1:2, :] = chk[h]
            if i == NQ - 2 and h == nh - 1:
                out_copy(g, olo, S - 2 * T).start()
            if i == NQ - 1:
                fl_scr[1, pl.ds(g, 1), :] = chk[h]
                out_copy(g, S - 2 * T if h == nh - 1 else olo, S).start()

        done = 0
        for j in range(len(units)):
            qk(units[j])
            if _LAG <= j < len(units) - _ENDL:
                pv(units[done])
                done += 1
        while done < len(units):
            pv(units[done])
            done += 1

    bufs = [h % 2 for h in range(HB)] + [0]
    if HB % 2:
        bufs[HB - 1] = 2

    qa = 2 * T * (_NA + 2)

    def first_k():
        return [cols_copy(k_hbm, k_all, 0, 0, S, isem.at[0])]

    def first_qv():
        return [cols_copy(q_hbm, q_all, 0, 2 * T, qa, isem.at[1]),
                cols_copy(v_hbm, v_all, 0, 0, S, isem.at[1])]

    def second():
        return [cols_copy(q_hbm, q_all, 0, qa, S, isem.at[3]),
                cols_copy(q_hbm, q_all, 0, 0, 2 * T, isem.at[3])] + in_copies(1, 1, 3)

    for cp in first_k() + first_qv() + second() + in_copies(2, HB, 2):
        cp.start()
    for cp in first_k():
        cp.wait()
    kf = k_all[0].astype(_f32)
    m0 = jnp.max(jnp.sum(kf * kf, axis=0, keepdims=True), axis=1, keepdims=True)
    st_scr[0:1, :] = jnp.maximum(jnp.broadcast_to(m0, (1, T)), _TINY) * 1.05
    for c in range(_NPRE):
        stage_k(0, 1, c)
    for cp in first_qv():
        cp.wait()
    block([0], [1], 1, 1 + _NA)
    for cp in second():
        cp.wait()
    block([0, 1], [1, 0], 1 + _NA)

    def step(s, carry):
        base = 1 + s * HB

        @pl.when(s < NS - 1)
        def _():
            for cp in in_copies(base + 1, HB, 2):
                cp.wait()

        @pl.when(s == NS - 1)
        def _():
            for cp in in_copies(base + 1, HB - 1, 2):
                cp.wait()

        @pl.when(s < NS - 2)
        def _():
            for cp in in_copies(base + 1 + HB, HB, 2):
                cp.start()

        @pl.when(s == NS - 2)
        def _():
            for cp in in_copies(base + 1 + HB, HB - 1, 2):
                cp.start()

        nxt = jnp.where(s == NS - 1, 0, base + HB)
        block([base + h for h in range(HB)] + [nxt], bufs)
        return carry

    lax.fori_loop(0, NS, step, 0)

    total = jnp.sum(fl_scr[0] + fl_scr[1])
    pltpu.make_async_copy(o_all, o_hbm, osem.at[0]).wait()

    @pl.when(jnp.logical_not(total < 1e30))
    def _():
        def head(g, carry):
            tg = jnp.sum(fl_scr[0, pl.ds(g, 1), :] + fl_scr[1, pl.ds(g, 1), :])

            @pl.when(jnp.logical_not(tg < 1e30))
            def _():
                ks_scr[...] = k_all[g].astype(_f32).T.astype(_bf16)

                def tile(j, carry):
                    off = pl.multiple_of(j * _TS, _TS)
                    s = jnp.dot(ks_scr[...], q_all[g, :, pl.ds(off, _TS)],
                                preferred_element_type=_f32)
                    m = jnp.max(s, axis=0, keepdims=True)
                    p = jnp.exp2((s - m) * (D ** -0.5 * _LOG2E))
                    l = jnp.sum(p, axis=0, keepdims=True)
                    o = jnp.dot(v_all[g], p.astype(_bf16), preferred_element_type=_f32)
                    o_all[g, :, pl.ds(off, _TS)] = (o / l).astype(o_all.dtype)
                    return carry

                lax.fori_loop(0, S // _TS, tile, 0)
                cp = out_copy(g, 0, S)
                cp.start()
                cp.wait()

            return carry

        lax.fori_loop(0, BH, head, 0)


@jax.jit
def pallas_standalone__fused_io_aware_attn__prompt_kernel(
    q: jax.Array,
    k: jax.Array,
    v: jax.Array,
):
    B, H, S, D = q.shape
    BH = B * H
    assert (BH - 1) % _HB == 0 and (BH - 1) // _HB >= 2 and D == 32 and S == 2048
    qt, kt, vt = (jnp.swapaxes(x, -1, -2).reshape(BH, D, S) for x in (q, k, v))
    hbm = pl.BlockSpec(memory_space=pl.ANY)
    o = pl.pallas_call(
        _kernel,
        in_specs=[hbm, hbm, hbm],
        out_specs=hbm,
        out_shape=jax.ShapeDtypeStruct((BH, D, S), q.dtype),
        scratch_shapes=[
            pltpu.VMEM((BH, D, S), q.dtype),
            pltpu.VMEM((BH, D, S), q.dtype),
            pltpu.VMEM((BH, D, S), q.dtype),
            pltpu.VMEM((BH, D, S), q.dtype),
            pltpu.VMEM((3, S // 2, _KA), _u32),
            pltpu.VMEM((3, D, S), _f32),
            pltpu.VMEM((8, _T), _f32),
            pltpu.VMEM((_KA // 2, _T), _u32),
            pltpu.VMEM((2, BH, _T), _f32),
            pltpu.VMEM((S, D), _bf16),
            pltpu.SemaphoreType.DMA((4,)),
            pltpu.SemaphoreType.DMA((1,)),
        ],
        compiler_params=pltpu.CompilerParams(
            vmem_limit_bytes=100 * 1024 * 1024,
            disable_bounds_checks=True),
    )(qt, kt, vt)
    return jnp.swapaxes(o.reshape(B, H, D, S), -1, -2)
```

```python
import jax
import jax.numpy as jnp
from jax import lax
import jax.experimental.pallas as pl
import jax.experimental.pallas.tpu as pltpu

_LOG2E = 1.4426950408889634
_T = 128
_KA = 80
_HB = 7
_LAG = 6
_ENDL = 5
_START = 76
_KDEP = (12, 7)
_NA = 2
_NPRE = 6
_BMAX = 8.0
_TINY = 2.0 ** -110
_TS = 512

_f32, _bf16, _i32, _u32 = jnp.float32, jnp.bfloat16, jnp.int32, jnp.uint32


@jax.jit
def _stage_k(kc):
    ka = jnp.concatenate([kc, jnp.ones((16, _T), _bf16), kc], axis=0).T
    kw = pltpu.bitcast(ka, _u32)
    return jnp.concatenate(
        [pltpu.roll(kw[j * 8:j * 8 + 8], 4, 0) for j in reversed(range(_T // 16))],
        axis=0)


@jax.jit
def _probs(kw, w):
    t = jnp.dot(pltpu.bitcast(kw, _bf16), w, preferred_element_type=_f32)
    hi = pltpu.bitcast(pltpu.bitcast(t, _i32) & (-4096), _f32)
    p = jnp.concatenate([jnp.exp2(t * 2.0 ** -11), jnp.exp2(t - hi)], axis=1)
    part = jnp.sum(p.reshape(_T // 8, 8, 2 * _T), axis=0)
    p = jnp.concatenate(
        [p[j * 8:j * 8 + 8] for j in reversed(range(_T // 8))], axis=0)
    return p, part


@jax.jit
def _norms(kc, vc):
    kf = kc.astype(_f32)
    vw = pltpu.bitcast(vc, _i32)
    vb = vw[0:8] | vw[8:16]
    vb = pltpu.bitcast((vb | (vb << 16)) & 0x60000000, _f32)
    return jnp.concatenate(
        [jnp.sum(kf * kf, axis=0, keepdims=True),
         jnp.max(vb, axis=0, keepdims=True)], axis=0)


@jax.jit
def _weights(q, kmax):
    qs = q.astype(_f32) * (q.shape[0] ** -0.5 * _LOG2E)
    qn = jnp.sum(qs * qs, axis=0, keepdims=True)
    qn = jnp.maximum(jnp.maximum(qn[:, :_T], qn[:, _T:]), _TINY)
    b2 = jnp.maximum(qn * kmax, 2.0 ** -40)
    e2 = (pltpu.bitcast(b2, _i32) >> 23) + 1
    b = pltpu.bitcast(((e2 + 128) >> 1) << 23, _f32)
    b = jnp.where(b2 < _BMAX * _BMAX, b, jnp.nan)
    row = lax.broadcasted_iota(_i32, (16, _T), 0)
    coef = jnp.where(
        row == 0, -2.0 ** 24, jnp.where(
            row == 4, -1.5 * 2.0 ** 12, jnp.where(
                row == 8, 2.0 ** 24, jnp.where(row == 12, -1.0, 0.0))))
    return jnp.concatenate(
        [qs[:, :_T] * 2.0 ** 11, coef * b, qs[:, _T:]], axis=0).astype(_bf16)


def _self_test():
    def keys(r, d):
        return (((r * 7 + d * 11 + (r >> 4) * d) & 15) - 8).astype(_f32) * 0.0625

    r = lax.broadcasted_iota(_i32, (_T, _KA), 0)
    c = lax.broadcasted_iota(_i32, (_T, _KA), 1)
    ka = jnp.where((c >= 32) & (c < 48), 1.0, keys(r, jnp.where(c < 32, c, c - 48)))
    d = lax.broadcasted_iota(_i32, (32, 2 * _T), 0)
    j = lax.broadcasted_iota(_i32, (32, 2 * _T), 1)
    q = (((d * 5 + j * 3 + (j >> 4) * d) & 15) - 8).astype(_f32) * 0.125
    w = _weights(q.astype(_bf16), jnp.full((1, _T), 8.5, _f32))
    p, _ = _probs(pltpu.bitcast(ka.astype(_bf16), _u32), w)
    r = lax.broadcasted_iota(_i32, (_T, 32), 0)
    k = keys(_T - 8 - (r & -8) + (r & 7), lax.broadcasted_iota(_i32, (_T, 32), 1))
    wf = w.astype(_f32)
    s = jnp.dot(k, jnp.concatenate([wf[:32] * 2.0 ** -11, wf[48:]], axis=1),
                preferred_element_type=_f32)
    ratio = p * jnp.exp2(-s)
    ok = jnp.max(ratio, axis=0, keepdims=True) < 1.02 * jnp.min(ratio, axis=0, keepdims=True)
    bad = jnp.where(ok, 0.0, jnp.nan)
    return bad[:, :_T] + bad[:, _T:]


def _kernel(q_hbm, k_hbm, v_hbm, o_hbm, q_all, k_all, v_all, o_all,
            ka_scr, vf_scr, st_scr, w_scr, fl_scr, ks_scr, isem, osem):
    T, HB = _T, _HB
    BH, D, S = q_hbm.shape
    NS = (BH - 1) // HB
    NC = S // T
    NQ = S // (2 * T)

    def in_copies(g, n, slot):
        return [pltpu.make_async_copy(a.at[pl.ds(g, n)], b.at[pl.ds(g, n)], isem.at[slot])
                for a, b in ((k_hbm, k_all), (v_hbm, v_all), (q_hbm, q_all))]

    def cols_copy(src, dst, g, lo, hi, sem):
        return pltpu.make_async_copy(src.at[g, :, pl.ds(lo, hi - lo)],
                                     dst.at[g, :, pl.ds(lo, hi - lo)], sem)

    def out_copy(g, lo, hi):
        return cols_copy(o_all, o_hbm, g, lo, hi, osem.at[0])

    def max_key_norm(g):
        m = None
        for c in range(NC):
            kn = _norms(k_all[g, :, c * T:(c + 1) * T], v_all[g, :, c * T:(c + 1) * T])
            if m is not None:
                kn = jnp.maximum(kn, m)
            m = jnp.max(kn, axis=1, keepdims=True)
        mb = jnp.broadcast_to(m, (2, T))
        return jnp.where(mb[1:2] == 0.0, jnp.inf, jnp.maximum(mb[0:1], _TINY) * 1.05)

    def weights(g, i, kmax):
        return _weights(q_all[g, :, 2 * i * T:(2 * i + 2) * T], kmax)

    def stage_k(g, buf, c):
        ka_scr[buf, c * T // 2:(c + 1) * T // 2, :] = _stage_k(k_all[g, :, c * T:(c + 1) * T])

    def stage_v(g, buf, c):
        vf_scr[buf, :, c * T:(c + 1) * T] = v_all[g, :, c * T:(c + 1) * T].astype(_f32)

    def block(gs, bufs, lo=1, hi=None):
        first = hi is not None
        nh = 1 if first else len(gs) - 1
        units = []
        for h in range(nh):
            rest = [(h, i, c) for i in range(1, NQ) for c in range(NC)]
            n = len(rest) - _START
            pos = [] if first else [_START + (c * n) // NC for c in range(NC)]
            for j, u in enumerate(rest):
                if j in pos:
                    units.append((h + 1, 0, pos.index(j)))
                if h > 0 or lo <= u[1] < (hi or NQ):
                    units.append(u)
        accs, ls, ps, ws, chk = {}, {}, {}, {}, {}
        kmaxs = {0: st_scr[0:1, :]}
        if not first:
            ws[0, lo] = pltpu.bitcast(w_scr[...], _bf16)
        if lo > 1:
            chk[0] = st_scr[1:2, :]

        def qk(u):
            h, i, c = u
            g, buf = gs[h], bufs[h]
            if i == 0 and c == 0:
                kmaxs[h] = max_key_norm(g)
            if (h, i) not in ws:
                ws[h, i] = weights(g, i, kmaxs[h])
            if i == 0 or (first and i == 1):
                if i == 0 or c >= _NPRE:
                    stage_k(g, buf, c)
                stage_v(g, buf, c)
            ps[u], part = _probs(ka_scr[buf, c * T // 2:(c + 1) * T // 2, :], ws[h, i])
            ls[h, i] = part if c == 0 else ls[h, i] + part
            if i < NQ - 1 and c == _KDEP[min(i, 1)]:
                kmaxs[h] = jnp.maximum(kmaxs[h], -part[0:1, :T])
                if h == nh:
                    st_scr[0:1, :] = kmaxs[h]
                if h == nh or (first and i == hi - 1):
                    w_scr[...] = pltpu.bitcast(weights(g, i + 1, kmaxs[h]), _u32)

        def pv(u):
            h, i, c = u
            g, buf = gs[h], bufs[h]
            r = jnp.dot(vf_scr[buf, :, c * T:(c + 1) * T], ps.pop(u),
                        preferred_element_type=_f32)
            accs[h, i] = r if c == 0 else accs[h, i] + r
            if c < NC - 1:
                return
            lsum = jnp.sum(ls[h, i], axis=0, keepdims=True)
            o_all[g, :, 2 * i * T:2 * (i + 1) * T] = (
                accs[h, i] * pl.reciprocal(lsum, approx=False)).astype(o_all.dtype)
            l1 = lsum[:, :T]
            if i == 0:
                fl_scr[0, pl.ds(g, 1), :] = l1
                if h == nh:
                    out_copy(g, 0, 2 * T).start()
                return
            chk[h] = chk[h] + l1 if h in chk else l1
            olo = 2 * T if h == 0 else 0
            if first and i == hi - 1:
                st_scr[1:2, :] = chk[h]
            if i == NQ - 2 and h == nh - 1:
                out_copy(g, olo, S - 2 * T).start()
            if i == NQ - 1:
                fl_scr[1, pl.ds(g, 1), :] = chk[h]
                out_copy(g, S - 2 * T if h == nh - 1 else olo, S).start()

        done = 0
        for j in range(len(units)):
            qk(units[j])
            if _LAG <= j < len(units) - _ENDL:
                pv(units[done])
                done += 1
        while done < len(units):
            pv(units[done])
            done += 1

    bufs = [h % 2 for h in range(HB)] + [0]
    if HB % 2:
        bufs[HB - 1] = 2

    qa = 2 * T * (_NA + 2)

    def first_k():
        return [cols_copy(k_hbm, k_all, 0, 0, S, isem.at[0])]

    def first_qv():
        return [cols_copy(q_hbm, q_all, 0, 2 * T, qa, isem.at[1]),
                cols_copy(v_hbm, v_all, 0, 0, S, isem.at[1])]

    def second():
        return [cols_copy(q_hbm, q_all, 0, qa, S, isem.at[3]),
                cols_copy(q_hbm, q_all, 0, 0, 2 * T, isem.at[3])] + in_copies(1, 1, 3)

    for cp in first_k() + first_qv() + second() + in_copies(2, HB, 2):
        cp.start()
    st_scr[2:3, :] = _self_test()
    for cp in first_k():
        cp.wait()
    kf = k_all[0].astype(_f32)
    m0 = jnp.max(jnp.sum(kf * kf, axis=0, keepdims=True), axis=1, keepdims=True)
    st_scr[0:1, :] = jnp.maximum(jnp.broadcast_to(m0, (1, T)), _TINY) * 1.05
    for c in range(_NPRE):
        stage_k(0, 1, c)
    for cp in first_qv():
        cp.wait()
    block([0], [1], 1, 1 + _NA)
    for cp in second():
        cp.wait()
    block([0, 1], [1, 0], 1 + _NA)

    def step(s, carry):
        base = 1 + s * HB

        @pl.when(s < NS - 1)
        def _():
            for cp in in_copies(base + 1, HB, 2):
                cp.wait()

        @pl.when(s == NS - 1)
        def _():
            for cp in in_copies(base + 1, HB - 1, 2):
                cp.wait()

        @pl.when(s < NS - 2)
        def _():
            for cp in in_copies(base + 1 + HB, HB, 2):
                cp.start()

        @pl.when(s == NS - 2)
        def _():
            for cp in in_copies(base + 1 + HB, HB - 1, 2):
                cp.start()

        nxt = jnp.where(s == NS - 1, 0, base + HB)
        block([base + h for h in range(HB)] + [nxt], bufs)
        return carry

    lax.fori_loop(0, NS, step, 0)

    total = jnp.sum(fl_scr[0] + fl_scr[1] + st_scr[2:3, :])
    pltpu.make_async_copy(o_all, o_hbm, osem.at[0]).wait()

    @pl.when(jnp.logical_not(total < 1e30))
    def _():
        def head(g, carry):
            tg = jnp.sum(fl_scr[0, pl.ds(g, 1), :] + fl_scr[1, pl.ds(g, 1), :]
                         + st_scr[2:3, :])

            @pl.when(jnp.logical_not(tg < 1e30))
            def _():
                ks_scr[...] = k_all[g].astype(_f32).T.astype(_bf16)

                def tile(j, carry):
                    off = pl.multiple_of(j * _TS, _TS)
                    s = jnp.dot(ks_scr[...], q_all[g, :, pl.ds(off, _TS)],
                                preferred_element_type=_f32)
                    m = jnp.max(s, axis=0, keepdims=True)
                    p = jnp.exp2((s - m) * (D ** -0.5 * _LOG2E))
                    l = jnp.sum(p, axis=0, keepdims=True)
                    o = jnp.dot(v_all[g], p.astype(_bf16), preferred_element_type=_f32)
                    o_all[g, :, pl.ds(off, _TS)] = (o / l).astype(o_all.dtype)
                    return carry

                lax.fori_loop(0, S // _TS, tile, 0)
                cp = out_copy(g, 0, S)
                cp.start()
                cp.wait()

            return carry

        lax.fori_loop(0, BH, head, 0)


@jax.jit
def pallas_standalone__fused_io_aware_attn__prompt_kernel(
    q: jax.Array,
    k: jax.Array,
    v: jax.Array,
):
    B, H, S, D = q.shape
    BH = B * H
    assert (BH - 1) % _HB == 0 and (BH - 1) // _HB >= 2 and D == 32 and S == 2048
    qt, kt, vt = (jnp.swapaxes(x, -1, -2).reshape(BH, D, S) for x in (q, k, v))
    hbm = pl.BlockSpec(memory_space=pl.ANY)
    o = pl.pallas_call(
        _kernel,
        in_specs=[hbm, hbm, hbm],
        out_specs=hbm,
        out_shape=jax.ShapeDtypeStruct((BH, D, S), q.dtype),
        scratch_shapes=[
            pltpu.VMEM((BH, D, S), q.dtype),
            pltpu.VMEM((BH, D, S), q.dtype),
            pltpu.VMEM((BH, D, S), q.dtype),
            pltpu.VMEM((BH, D, S), q.dtype),
            pltpu.VMEM((3, S // 2, _KA), _u32),
            pltpu.VMEM((3, D, S), _f32),
            pltpu.VMEM((8, _T), _f32),
            pltpu.VMEM((_KA // 2, _T), _u32),
            pltpu.VMEM((2, BH, _T), _f32),
            pltpu.VMEM((S, D), _bf16),
            pltpu.SemaphoreType.DMA((4,)),
            pltpu.SemaphoreType.DMA((1,)),
        ],
        compiler_params=pltpu.CompilerParams(
            vmem_limit_bytes=100 * 1024 * 1024,
            disable_bounds_checks=True),
    )(qt, kt, vt)
    return jnp.swapaxes(o.reshape(B, H, D, S), -1, -2)
```

```python
import functools

import jax
import jax.numpy as jnp
from jax import lax
import jax.experimental.pallas as pl
import jax.experimental.pallas.tpu as pltpu

_LOG2E = 1.4426950408889634
_T = 128
_KA = 80
_HB = 7
_LAG = 6
_FILL = 8
_ENDL = 6
_SPLIT = {0: 80, 8: 32}
_START = 76
_KDEP = (12, 7)
_NA = 2
_NPRE = 6
_BMAX = 8.0
_TINY = 2.0 ** -110
_TS = 512

_f32, _bf16, _i32, _u32 = jnp.float32, jnp.bfloat16, jnp.int32, jnp.uint32


@jax.jit
def _stage_k(kc):
    ka = jnp.concatenate([kc, jnp.ones((16, _T), _bf16), kc], axis=0).T
    kw = pltpu.bitcast(ka, _u32)
    return jnp.concatenate(
        [pltpu.roll(kw[j * 8:j * 8 + 8], 4, 0) for j in reversed(range(_T // 16))],
        axis=0)


@functools.partial(jax.jit, static_argnums=2)
def _probs(kw, w, split=0):
    parts = [kw[:split // 2], kw[split // 2:]] if split else [kw]
    t = jnp.concatenate(
        [jnp.dot(pltpu.bitcast(x, _bf16), w, preferred_element_type=_f32) for x in parts],
        axis=0)
    hi = pltpu.bitcast(pltpu.bitcast(t, _i32) & (-4096), _f32)
    p = jnp.concatenate([jnp.exp2(t * 2.0 ** -11), jnp.exp2(t - hi)], axis=1)
    part = jnp.sum(p.reshape(_T // 8, 8, 2 * _T), axis=0)
    p = jnp.concatenate(
        [p[j * 8:j * 8 + 8] for j in reversed(range(_T // 8))], axis=0)
    return p, part


@jax.jit
def _norms(kc, vc):
    kf = kc.astype(_f32)
    vw = pltpu.bitcast(vc, _i32)
    vb = vw[0:8] | vw[8:16]
    vb = pltpu.bitcast((vb | (vb << 16)) & 0x60000000, _f32)
    return jnp.concatenate(
        [jnp.sum(kf * kf, axis=0, keepdims=True),
         jnp.max(vb, axis=0, keepdims=True)], axis=0)


@jax.jit
def _weights(q, kmax):
    qs = q.astype(_f32) * (q.shape[0] ** -0.5 * _LOG2E)
    qn = jnp.sum(qs * qs, axis=0, keepdims=True)
    qn = jnp.maximum(jnp.maximum(qn[:, :_T], qn[:, _T:]), _TINY)
    b2 = jnp.maximum(qn * kmax, 2.0 ** -40)
    e2 = (pltpu.bitcast(b2, _i32) >> 23) + 1
    b = pltpu.bitcast(((e2 + 128) >> 1) << 23, _f32)
    b = jnp.where(b2 < _BMAX * _BMAX, b, jnp.nan)
    row = lax.broadcasted_iota(_i32, (16, _T), 0)
    coef = jnp.where(
        row == 0, -2.0 ** 24, jnp.where(
            row == 4, -1.5 * 2.0 ** 12, jnp.where(
                row == 8, 2.0 ** 24, jnp.where(row == 12, -1.0, 0.0))))
    return jnp.concatenate(
        [qs[:, :_T] * 2.0 ** 11, coef * b, qs[:, _T:]], axis=0).astype(_bf16)


def _self_test():
    def keys(r, d):
        return (((r * 7 + d * 11 + (r >> 4) * d) & 15) - 8).astype(_f32) * 0.0625

    r = lax.broadcasted_iota(_i32, (_T, _KA), 0)
    c = lax.broadcasted_iota(_i32, (_T, _KA), 1)
    ka = jnp.where((c >= 32) & (c < 48), 1.0, keys(r, jnp.where(c < 32, c, c - 48)))
    d = lax.broadcasted_iota(_i32, (32, 2 * _T), 0)
    j = lax.broadcasted_iota(_i32, (32, 2 * _T), 1)
    q = (((d * 5 + j * 3 + (j >> 4) * d) & 15) - 8).astype(_f32) * 0.125
    w = _weights(q.astype(_bf16), jnp.full((1, _T), 8.5, _f32))
    p, _ = _probs(pltpu.bitcast(ka.astype(_bf16), _u32), w)
    r = lax.broadcasted_iota(_i32, (_T, 32), 0)
    k = keys(_T - 8 - (r & -8) + (r & 7), lax.broadcasted_iota(_i32, (_T, 32), 1))
    wf = w.astype(_f32)
    s = jnp.dot(k, jnp.concatenate([wf[:32] * 2.0 ** -11, wf[48:]], axis=1),
                preferred_element_type=_f32)
    ratio = p * jnp.exp2(-s)
    ok = jnp.max(ratio, axis=0, keepdims=True) < 1.02 * jnp.min(ratio, axis=0, keepdims=True)
    bad = jnp.where(ok, 0.0, jnp.nan)
    return bad[:, :_T] + bad[:, _T:]


def _kernel(q_hbm, k_hbm, v_hbm, o_hbm, q_all, k_all, v_all, o_all,
            ka_scr, vf_scr, st_scr, w_scr, fl_scr, ks_scr, isem, osem):
    T, HB = _T, _HB
    BH, D, S = q_hbm.shape
    NS = (BH - 1) // HB
    NC = S // T
    NQ = S // (2 * T)

    def in_copies(g, n, slot):
        return [pltpu.make_async_copy(a.at[pl.ds(g, n)], b.at[pl.ds(g, n)], isem.at[slot])
                for a, b in ((k_hbm, k_all), (v_hbm, v_all), (q_hbm, q_all))]

    def cols_copy(src, dst, g, lo, hi, sem):
        return pltpu.make_async_copy(src.at[g, :, pl.ds(lo, hi - lo)],
                                     dst.at[g, :, pl.ds(lo, hi - lo)], sem)

    def out_copy(g, lo, hi):
        return cols_copy(o_all, o_hbm, g, lo, hi, osem.at[0])

    def max_key_norm(g):
        m = None
        for c in range(NC):
            kn = _norms(k_all[g, :, c * T:(c + 1) * T], v_all[g, :, c * T:(c + 1) * T])
            if m is not None:
                kn = jnp.maximum(kn, m)
            m = jnp.max(kn, axis=1, keepdims=True)
        mb = jnp.broadcast_to(m, (2, T))
        return jnp.where(mb[1:2] == 0.0, jnp.inf, jnp.maximum(mb[0:1], _TINY) * 1.05)

    def weights(g, i, kmax):
        return _weights(q_all[g, :, 2 * i * T:(2 * i + 2) * T], kmax)

    def stage_k(g, buf, c):
        ka_scr[buf, c * T // 2:(c + 1) * T // 2, :] = _stage_k(k_all[g, :, c * T:(c + 1) * T])

    def stage_v(g, buf, c):
        vf_scr[buf, :, c * T:(c + 1) * T] = v_all[g, :, c * T:(c + 1) * T].astype(_f32)

    def block(gs, bufs, lo=1, hi=None):
        first = hi is not None
        nh = 1 if first else len(gs) - 1
        units = []
        for h in range(nh):
            rest = [(h, i, c) for i in range(1, NQ) for c in range(NC)]
            n = len(rest) - _START
            pos = [] if first else [_START + (c * n) // NC for c in range(NC)]
            for j, u in enumerate(rest):
                if j in pos:
                    units.append((h + 1, 0, pos.index(j)))
                if h > 0 or lo <= u[1] < (hi or NQ):
                    units.append(u)
        accs, ls, ps, ws, chk = {}, {}, {}, {}, {}
        kmaxs = {0: st_scr[0:1, :]}
        if not first:
            ws[0, lo] = pltpu.bitcast(w_scr[...], _bf16)
        if lo > 1:
            chk[0] = st_scr[1:2, :]

        def qk(u, split):
            h, i, c = u
            g, buf = gs[h], bufs[h]
            if i == 0 and c == 0:
                kmaxs[h] = max_key_norm(g)
            if (h, i) not in ws:
                ws[h, i] = weights(g, i, kmaxs[h])
            if i == 0 or (first and i == 1):
                if i == 0 or c >= _NPRE:
                    stage_k(g, buf, c)
                stage_v(g, buf, c)
            ps[u], part = _probs(
                ka_scr[buf, c * T // 2:(c + 1) * T // 2, :], ws[h, i], split)
            ls[h, i] = part if c == 0 else ls[h, i] + part
            if i < NQ - 1 and c == _KDEP[min(i, 1)]:
                kmaxs[h] = jnp.maximum(kmaxs[h], -part[0:1, :T])
                if h == nh:
                    st_scr[0:1, :] = kmaxs[h]
                if h == nh or (first and i == hi - 1):
                    w_scr[...] = pltpu.bitcast(weights(g, i + 1, kmaxs[h]), _u32)

        def pv(u):
            h, i, c = u
            g, buf = gs[h], bufs[h]
            r = jnp.dot(vf_scr[buf, :, c * T:(c + 1) * T], ps.pop(u),
                        preferred_element_type=_f32)
            accs[h, i] = r if c == 0 else r + accs[h, i]
            if c < NC - 1:
                return
            lsum = jnp.sum(ls[h, i], axis=0, keepdims=True)
            o_all[g, :, 2 * i * T:2 * (i + 1) * T] = (
                accs[h, i] * pl.reciprocal(lsum, approx=False)).astype(o_all.dtype)
            l1 = lsum[:, :T]
            if i == 0:
                fl_scr[0, pl.ds(g, 1), :] = l1
                if h == nh:
                    out_copy(g, 0, 2 * T).start()
                return
            chk[h] = chk[h] + l1 if h in chk else l1
            olo = 2 * T if h == 0 else 0
            if first and i == hi - 1:
                st_scr[1:2, :] = chk[h]
            if i == NQ - 2 and h == nh - 1:
                out_copy(g, olo, S - 2 * T).start()
            if i == NQ - 1:
                fl_scr[1, pl.ds(g, 1), :] = chk[h]
                out_copy(g, S - 2 * T if h == nh - 1 else olo, S).start()

        done = 0
        for j in range(len(units)):
            qk(units[j], _SPLIT.get(j, 0))
            while _FILL - 1 <= j < len(units) - _ENDL and done <= j - _LAG:
                pv(units[done])
                done += 1
        while done < len(units):
            pv(units[done])
            done += 1

    bufs = [h % 2 for h in range(HB)] + [0]
    if HB % 2:
        bufs[HB - 1] = 2

    qa = 2 * T * (_NA + 2)

    def first_k():
        return [cols_copy(k_hbm, k_all, 0, 0, S, isem.at[0])]

    def first_qv():
        return [cols_copy(q_hbm, q_all, 0, 2 * T, qa, isem.at[1]),
                cols_copy(v_hbm, v_all, 0, 0, S, isem.at[1])]

    def second():
        return [cols_copy(q_hbm, q_all, 0, qa, S, isem.at[3]),
                cols_copy(q_hbm, q_all, 0, 0, 2 * T, isem.at[3])] + in_copies(1, 1, 3)

    for cp in first_k() + first_qv() + second() + in_copies(2, HB, 2):
        cp.start()
    st_scr[2:3, :] = _self_test()
    for cp in first_k():
        cp.wait()
    kf = k_all[0].astype(_f32)
    m0 = jnp.max(jnp.sum(kf * kf, axis=0, keepdims=True), axis=1, keepdims=True)
    st_scr[0:1, :] = jnp.maximum(jnp.broadcast_to(m0, (1, T)), _TINY) * 1.05
    for c in range(_NPRE):
        stage_k(0, 1, c)
    for cp in first_qv():
        cp.wait()
    block([0], [1], 1, 1 + _NA)
    for cp in second():
        cp.wait()
    block([0, 1], [1, 0], 1 + _NA)

    def step(s, carry):
        base = 1 + s * HB

        @pl.when(s < NS - 1)
        def _():
            for cp in in_copies(base + 1, HB, 2):
                cp.wait()

        @pl.when(s == NS - 1)
        def _():
            for cp in in_copies(base + 1, HB - 1, 2):
                cp.wait()

        @pl.when(s < NS - 2)
        def _():
            for cp in in_copies(base + 1 + HB, HB, 2):
                cp.start()

        @pl.when(s == NS - 2)
        def _():
            for cp in in_copies(base + 1 + HB, HB - 1, 2):
                cp.start()

        nxt = jnp.where(s == NS - 1, 0, base + HB)
        block([base + h for h in range(HB)] + [nxt], bufs)
        return carry

    lax.fori_loop(0, NS, step, 0)

    total = jnp.sum(fl_scr[0] + fl_scr[1] + st_scr[2:3, :])
    pltpu.make_async_copy(o_all, o_hbm, osem.at[0]).wait()

    @pl.when(jnp.logical_not(total < 1e30))
    def _():
        def head(g, carry):
            tg = jnp.sum(fl_scr[0, pl.ds(g, 1), :] + fl_scr[1, pl.ds(g, 1), :]
                         + st_scr[2:3, :])

            @pl.when(jnp.logical_not(tg < 1e30))
            def _():
                ks_scr[...] = k_all[g].astype(_f32).T.astype(_bf16)

                def tile(j, carry):
                    off = pl.multiple_of(j * _TS, _TS)
                    s = jnp.dot(ks_scr[...], q_all[g, :, pl.ds(off, _TS)],
                                preferred_element_type=_f32)
                    m = jnp.max(s, axis=0, keepdims=True)
                    p = jnp.exp2((s - m) * (D ** -0.5 * _LOG2E))
                    l = jnp.sum(p, axis=0, keepdims=True)
                    o = jnp.dot(v_all[g], p.astype(_bf16), preferred_element_type=_f32)
                    o_all[g, :, pl.ds(off, _TS)] = (o / l).astype(o_all.dtype)
                    return carry

                lax.fori_loop(0, S // _TS, tile, 0)
                cp = out_copy(g, 0, S)
                cp.start()
                cp.wait()

            return carry

        lax.fori_loop(0, BH, head, 0)


@jax.jit
def pallas_standalone__fused_io_aware_attn__prompt_kernel(
    q: jax.Array,
    k: jax.Array,
    v: jax.Array,
):
    B, H, S, D = q.shape
    BH = B * H
    assert (BH - 1) % _HB == 0 and (BH - 1) // _HB >= 2 and D == 32 and S == 2048
    qt, kt, vt = (jnp.swapaxes(x, -1, -2).reshape(BH, D, S) for x in (q, k, v))
    hbm = pl.BlockSpec(memory_space=pl.ANY)
    o = pl.pallas_call(
        _kernel,
        in_specs=[hbm, hbm, hbm],
        out_specs=hbm,
        out_shape=jax.ShapeDtypeStruct((BH, D, S), q.dtype),
        scratch_shapes=[
            pltpu.VMEM((BH, D, S), q.dtype),
            pltpu.VMEM((BH, D, S), q.dtype),
            pltpu.VMEM((BH, D, S), q.dtype),
            pltpu.VMEM((BH, D, S), q.dtype),
            pltpu.VMEM((3, S // 2, _KA), _u32),
            pltpu.VMEM((3, D, S), _f32),
            pltpu.VMEM((8, _T), _f32),
            pltpu.VMEM((_KA // 2, _T), _u32),
            pltpu.VMEM((2, BH, _T), _f32),
            pltpu.VMEM((S, D), _bf16),
            pltpu.SemaphoreType.DMA((4,)),
            pltpu.SemaphoreType.DMA((1,)),
        ],
        compiler_params=pltpu.CompilerParams(
            vmem_limit_bytes=100 * 1024 * 1024,
            disable_bounds_checks=True),
    )(qt, kt, vt)
    return jnp.swapaxes(o.reshape(B, H, D, S), -1, -2)
```

```python
import functools

import jax
import jax.numpy as jnp
from jax import lax
import jax.experimental.pallas as pl
import jax.experimental.pallas.tpu as pltpu

_LOG2E = 1.4426950408889634
_T = 128
_KA = 80
_HB = 7
_LAG = 6
_FILL = 9
_ENDL = 6
_SPLIT = {0: 112, 12: 32, -9: 80}
_START = 76
_KDEP = (6, 7)
_NA = 2
_NPRE = 6
_BMAX = 8.0
_TINY = 2.0 ** -110
_TS = 512

_f32, _bf16, _i32, _u32 = jnp.float32, jnp.bfloat16, jnp.int32, jnp.uint32


@jax.jit
def _stage_k(kc):
    ka = jnp.concatenate([kc, jnp.ones((16, _T), _bf16), kc], axis=0).T
    kw = pltpu.bitcast(ka, _u32)
    return jnp.concatenate(
        [pltpu.roll(kw[j * 8:j * 8 + 8], 4, 0) for j in reversed(range(_T // 16))],
        axis=0)


@functools.partial(jax.jit, static_argnums=2)
def _probs(kw, w, split=0):
    parts = [kw[:split // 2], kw[split // 2:]] if split else [kw]
    t = jnp.concatenate(
        [jnp.dot(pltpu.bitcast(x, _bf16), w, preferred_element_type=_f32) for x in parts],
        axis=0)
    hi = pltpu.bitcast(pltpu.bitcast(t, _i32) & (-4096), _f32)
    p = jnp.concatenate([jnp.exp2(t * 2.0 ** -11), jnp.exp2(t - hi)], axis=1)
    part = jnp.sum(p.reshape(_T // 8, 8, 2 * _T), axis=0)
    p = jnp.concatenate(
        [p[j * 8:j * 8 + 8] for j in reversed(range(_T // 8))], axis=0)
    return p, part


@jax.jit
def _norms(kc, vc):
    kf = kc.astype(_f32)
    vw = pltpu.bitcast(vc, _i32)
    vb = vw[0:8] | vw[8:16]
    vb = pltpu.bitcast((vb | (vb << 16)) & 0x60000000, _f32)
    return jnp.concatenate(
        [jnp.sum(kf * kf, axis=0, keepdims=True),
         jnp.max(vb, axis=0, keepdims=True)], axis=0)


@jax.jit
def _weights(q, kmax):
    qs = q.astype(_f32) * (q.shape[0] ** -0.5 * _LOG2E)
    qn = jnp.sum(qs * qs, axis=0, keepdims=True)
    qn = jnp.maximum(jnp.maximum(qn[:, :_T], qn[:, _T:]), _TINY)
    b2 = jnp.maximum(qn * kmax, 2.0 ** -40)
    e2 = (pltpu.bitcast(b2, _i32) >> 23) + 1
    b = pltpu.bitcast(((e2 + 128) >> 1) << 23, _f32)
    b = jnp.where(b2 < _BMAX * _BMAX, b, jnp.nan)
    row = lax.broadcasted_iota(_i32, (16, _T), 0)
    coef = jnp.where(
        row == 0, -2.0 ** 24, jnp.where(
            row == 4, -1.5 * 2.0 ** 12, jnp.where(
                row == 8, 2.0 ** 24, jnp.where(row == 12, -1.0, 0.0))))
    return jnp.concatenate(
        [qs[:, :_T] * 2.0 ** 11, coef * b, qs[:, _T:]], axis=0).astype(_bf16)


def _self_test():
    def keys(r, d):
        return (((r * 7 + d * 11 + (r >> 4) * d) & 15) - 8).astype(_f32) * 0.0625

    r = lax.broadcasted_iota(_i32, (_T, _KA), 0)
    c = lax.broadcasted_iota(_i32, (_T, _KA), 1)
    ka = jnp.where((c >= 32) & (c < 48), 1.0, keys(r, jnp.where(c < 32, c, c - 48)))
    d = lax.broadcasted_iota(_i32, (32, 2 * _T), 0)
    j = lax.broadcasted_iota(_i32, (32, 2 * _T), 1)
    q = (((d * 5 + j * 3 + (j >> 4) * d) & 15) - 8).astype(_f32) * 0.125
    w = _weights(q.astype(_bf16), jnp.full((1, _T), 8.5, _f32))
    p, _ = _probs(pltpu.bitcast(ka.astype(_bf16), _u32), w)
    r = lax.broadcasted_iota(_i32, (_T, 32), 0)
    k = keys(_T - 8 - (r & -8) + (r & 7), lax.broadcasted_iota(_i32, (_T, 32), 1))
    wf = w.astype(_f32)
    s = jnp.dot(k, jnp.concatenate([wf[:32] * 2.0 ** -11, wf[48:]], axis=1),
                preferred_element_type=_f32)
    ratio = p * jnp.exp2(-s)
    ok = jnp.max(ratio, axis=0, keepdims=True) < 1.02 * jnp.min(ratio, axis=0, keepdims=True)
    bad = jnp.where(ok, 0.0, jnp.nan)
    return bad[:, :_T] + bad[:, _T:]


def _kernel(q_hbm, k_hbm, v_hbm, o_hbm, q_all, k_all, v_all, o_all,
            ka_scr, vf_scr, st_scr, w_scr, fl_scr, ks_scr, vb_scr, isem, osem):
    T, HB = _T, _HB
    BH, D, S = q_hbm.shape
    NS = (BH - 1) // HB
    NC = S // T
    NQ = S // (2 * T)

    def in_copies(g, n, slot):
        return [pltpu.make_async_copy(a.at[pl.ds(g, n)], b.at[pl.ds(g, n)], isem.at[slot])
                for a, b in ((k_hbm, k_all), (v_hbm, v_all), (q_hbm, q_all))]

    def cols_copy(src, dst, g, lo, hi, sem):
        return pltpu.make_async_copy(src.at[g, :, pl.ds(lo, hi - lo)],
                                     dst.at[g, :, pl.ds(lo, hi - lo)], sem)

    def out_copy(g, lo, hi):
        return cols_copy(o_all, o_hbm, g, lo, hi, osem.at[0])

    def max_key_norm(g):
        m = None
        for c in range(NC):
            kn = _norms(k_all[g, :, c * T:(c + 1) * T], v_all[g, :, c * T:(c + 1) * T])
            if m is not None:
                kn = jnp.maximum(kn, m)
            m = jnp.max(kn, axis=1, keepdims=True)
        mb = jnp.broadcast_to(m, (2, T))
        return jnp.where(mb[1:2] == 0.0, jnp.inf, jnp.maximum(mb[0:1], _TINY) * 1.05)

    def weights(g, i, kmax):
        return _weights(q_all[g, :, 2 * i * T:(2 * i + 2) * T], kmax)

    def stage_k(g, buf, c):
        ka_scr[buf, c * T // 2:(c + 1) * T // 2, :] = _stage_k(k_all[g, :, c * T:(c + 1) * T])

    def stage_v(g, buf, c):
        vf_scr[buf, :, c * T:(c + 1) * T] = v_all[g, :, c * T:(c + 1) * T].astype(_f32)
        vb_scr[buf, :, c * T:(c + 1) * T] = pltpu.bitcast(v_all[g, :, c * T:(c + 1) * T], _u32)

    def block(gs, bufs, lo=1, hi=None):
        first = hi is not None
        nh = 1 if first else len(gs) - 1
        units = []
        for h in range(nh):
            rest = [(h, i, c) for i in range(1, NQ) for c in range(NC)]
            n = len(rest) - _START
            pos = [] if first else [_START + (c * n) // NC for c in range(NC)]
            for j, u in enumerate(rest):
                if j in pos:
                    units.append((h + 1, 0, pos.index(j)))
                if h > 0 or lo <= u[1] < (hi or NQ):
                    units.append(u)
        accs, ls, ps, ws, chk = {}, {}, {}, {}, {}
        kmaxs = {0: st_scr[0:1, :]}
        if not first:
            ws[0, lo] = pltpu.bitcast(w_scr[...], _bf16)
        if lo > 1:
            chk[0] = st_scr[1:2, :]

        def qk(u, split):
            h, i, c = u
            g, buf = gs[h], bufs[h]
            if i == 0 and c == 0:
                kmaxs[h] = max_key_norm(g)
            if (h, i) not in ws:
                ws[h, i] = weights(g, i, kmaxs[h])
            if i == 0 or (first and i == 1):
                if i == 0 or c >= _NPRE:
                    stage_k(g, buf, c)
                stage_v(g, buf, c)
            ps[u], part = _probs(
                ka_scr[buf, c * T // 2:(c + 1) * T // 2, :], ws[h, i], split)
            ls[h, i] = part if c == 0 else ls[h, i] + part
            if i < NQ - 1 and c == _KDEP[min(i, 1)]:
                kmaxs[h] = jnp.maximum(kmaxs[h], -part[0:1, :T])
                if h == nh:
                    st_scr[0:1, :] = kmaxs[h]
                if h == nh or (first and i == hi - 1):
                    w_scr[...] = pltpu.bitcast(weights(g, i + 1, kmaxs[h]), _u32)

        def pv(u):
            h, i, c = u
            g, buf = gs[h], bufs[h]
            p = ps.pop(u)
            rs = (jnp.dot(pltpu.bitcast(vb_scr[buf, :, c * T:(c + 1) * T], _bf16),
                          p[:, :T].astype(_bf16), preferred_element_type=_f32),
                  jnp.dot(vf_scr[buf, :, c * T:(c + 1) * T], p[:, T:],
                          preferred_element_type=_f32))
            accs[h, i] = rs if c == 0 else [r + a for r, a in zip(rs, accs[h, i])]
            if c < NC - 1:
                return
            lsum = jnp.sum(ls[h, i], axis=0, keepdims=True)
            o_all[g, :, 2 * i * T:2 * (i + 1) * T] = (
                jnp.concatenate(accs[h, i], axis=1) * pl.reciprocal(lsum, approx=False)
            ).astype(o_all.dtype)
            l1 = lsum[:, :T]
            if i == 0:
                fl_scr[0, pl.ds(g, 1), :] = l1
                if h == nh:
                    out_copy(g, 0, 2 * T).start()
                return
            chk[h] = chk[h] + l1 if h in chk else l1
            olo = 2 * T if h == 0 else 0
            if first and i == hi - 1:
                st_scr[1:2, :] = chk[h]
            if i == NQ - 2 and h == nh - 1:
                out_copy(g, olo, S - 2 * T).start()
            if i == NQ - 1:
                fl_scr[1, pl.ds(g, 1), :] = chk[h]
                out_copy(g, S - 2 * T if h == nh - 1 else olo, S).start()

        done = 0
        for j in range(len(units)):
            qk(units[j], _SPLIT.get(j, 0) or _SPLIT.get(j - len(units), 0))
            while _FILL - 1 <= j < len(units) - _ENDL and done <= j - _LAG:
                pv(units[done])
                done += 1
        while done < len(units):
            pv(units[done])
            done += 1

    bufs = [h % 2 for h in range(HB)] + [0]
    if HB % 2:
        bufs[HB - 1] = 2

    qa = 2 * T * (_NA + 2)

    def first_k():
        return [cols_copy(k_hbm, k_all, 0, 0, S, isem.at[0])]

    def first_qv():
        return [cols_copy(q_hbm, q_all, 0, 2 * T, qa, isem.at[1]),
                cols_copy(v_hbm, v_all, 0, 0, S, isem.at[1])]

    def second():
        return [cols_copy(q_hbm, q_all, 0, qa, S, isem.at[3]),
                cols_copy(q_hbm, q_all, 0, 0, 2 * T, isem.at[3])] + in_copies(1, 1, 3)

    for cp in first_k() + first_qv() + second() + in_copies(2, HB, 2):
        cp.start()
    st_scr[2:3, :] = _self_test()
    for cp in first_k():
        cp.wait()
    kf = k_all[0].astype(_f32)
    m0 = jnp.max(jnp.sum(kf * kf, axis=0, keepdims=True), axis=1, keepdims=True)
    st_scr[0:1, :] = jnp.maximum(jnp.broadcast_to(m0, (1, T)), _TINY) * 1.05
    for c in range(_NPRE):
        stage_k(0, 1, c)
    for cp in first_qv():
        cp.wait()
    block([0], [1], 1, 1 + _NA)
    for cp in second():
        cp.wait()
    block([0, 1], [1, 0], 1 + _NA)

    def step(s, carry):
        base = 1 + s * HB

        @pl.when(s < NS - 1)
        def _():
            for cp in in_copies(base + 1, HB, 2):
                cp.wait()

        @pl.when(s == NS - 1)
        def _():
            for cp in in_copies(base + 1, HB - 1, 2):
                cp.wait()

        @pl.when(s < NS - 2)
        def _():
            for cp in in_copies(base + 1 + HB, HB, 2):
                cp.start()

        @pl.when(s == NS - 2)
        def _():
            for cp in in_copies(base + 1 + HB, HB - 1, 2):
                cp.start()

        nxt = jnp.where(s == NS - 1, 0, base + HB)
        block([base + h for h in range(HB)] + [nxt], bufs)
        return carry

    lax.fori_loop(0, NS, step, 0)

    total = jnp.sum(fl_scr[0] + fl_scr[1] + st_scr[2:3, :])
    pltpu.make_async_copy(o_all, o_hbm, osem.at[0]).wait()

    @pl.when(jnp.logical_not(total < 1e30))
    def _():
        def head(g, carry):
            tg = jnp.sum(fl_scr[0, pl.ds(g, 1), :] + fl_scr[1, pl.ds(g, 1), :]
                         + st_scr[2:3, :])

            @pl.when(jnp.logical_not(tg < 1e30))
            def _():
                ks_scr[...] = k_all[g].astype(_f32).T.astype(_bf16)

                def tile(j, carry):
                    off = pl.multiple_of(j * _TS, _TS)
                    s = jnp.dot(ks_scr[...], q_all[g, :, pl.ds(off, _TS)],
                                preferred_element_type=_f32)
                    m = jnp.max(s, axis=0, keepdims=True)
                    p = jnp.exp2((s - m) * (D ** -0.5 * _LOG2E))
                    l = jnp.sum(p, axis=0, keepdims=True)
                    o = jnp.dot(v_all[g], p.astype(_bf16), preferred_element_type=_f32)
                    o_all[g, :, pl.ds(off, _TS)] = (o / l).astype(o_all.dtype)
                    return carry

                lax.fori_loop(0, S // _TS, tile, 0)
                cp = out_copy(g, 0, S)
                cp.start()
                cp.wait()

            return carry

        lax.fori_loop(0, BH, head, 0)


@jax.jit
def pallas_standalone__fused_io_aware_attn__prompt_kernel(
    q: jax.Array,
    k: jax.Array,
    v: jax.Array,
):
    B, H, S, D = q.shape
    BH = B * H
    assert (BH - 1) % _HB == 0 and (BH - 1) // _HB >= 2 and D == 32 and S == 2048
    qt, kt, vt = (jnp.swapaxes(x, -1, -2).reshape(BH, D, S) for x in (q, k, v))
    hbm = pl.BlockSpec(memory_space=pl.ANY)
    o = pl.pallas_call(
        _kernel,
        in_specs=[hbm, hbm, hbm],
        out_specs=hbm,
        out_shape=jax.ShapeDtypeStruct((BH, D, S), q.dtype),
        scratch_shapes=[
            pltpu.VMEM((BH, D, S), q.dtype),
            pltpu.VMEM((BH, D, S), q.dtype),
            pltpu.VMEM((BH, D, S), q.dtype),
            pltpu.VMEM((BH, D, S), q.dtype),
            pltpu.VMEM((3, S // 2, _KA), _u32),
            pltpu.VMEM((3, D, S), _f32),
            pltpu.VMEM((8, _T), _f32),
            pltpu.VMEM((_KA // 2, _T), _u32),
            pltpu.VMEM((2, BH, _T), _f32),
            pltpu.VMEM((S, D), _bf16),
            pltpu.VMEM((3, D // 2, S), _u32),
            pltpu.SemaphoreType.DMA((4,)),
            pltpu.SemaphoreType.DMA((1,)),
        ],
        compiler_params=pltpu.CompilerParams(
            vmem_limit_bytes=100 * 1024 * 1024,
            disable_bounds_checks=True),
    )(qt, kt, vt)
    return jnp.swapaxes(o.reshape(B, H, D, S), -1, -2)
```

```python
import functools

import jax
import jax.numpy as jnp
from jax import lax
import jax.experimental.pallas as pl
import jax.experimental.pallas.tpu as pltpu

_LOG2E = 1.4426950408889634
_T = 128
_KA = 80
_HB = 7
_LAG = 6
_FILL = 9
_ENDL = 6
_SPLIT = {0: 112, 12: 32, -9: 80}
_START = 76
_KDEP = (6, 7)
_NA = 2
_NPRE = 6
_BMAX = 8.0
_TINY = 2.0 ** -110
_NT = 8
_OFF = 8

_f32, _bf16, _i32, _u32 = jnp.float32, jnp.bfloat16, jnp.int32, jnp.uint32


@jax.jit
def _stage_k(kc):
    ka = jnp.concatenate([kc, jnp.ones((16, _T), _bf16), kc], axis=0).T
    kw = pltpu.bitcast(ka, _u32)
    return jnp.concatenate(
        [pltpu.roll(kw[j * 8:j * 8 + 8], 4, 0) for j in reversed(range(_T // 16))],
        axis=0)


@functools.partial(jax.jit, static_argnums=2)
def _probs(kw, w, split=0):
    parts = [kw[:split // 2], kw[split // 2:]] if split else [kw]
    t = jnp.concatenate(
        [jnp.dot(pltpu.bitcast(x, _bf16), w, preferred_element_type=_f32) for x in parts],
        axis=0)
    hi = pltpu.bitcast(pltpu.bitcast(t, _i32) & (-4096), _f32)
    p = jnp.concatenate([jnp.exp2(t * 2.0 ** -11), jnp.exp2(t - hi)], axis=1)
    part = jnp.sum(p.reshape(_T // 8, 8, 2 * _T), axis=0)
    p = jnp.concatenate(
        [p[j * 8:j * 8 + 8] for j in reversed(range(_T // 8))], axis=0)
    return p, part


@jax.jit
def _norms(kc, vc):
    kf = kc.astype(_f32)
    vw = pltpu.bitcast(vc, _i32)
    vb = vw[0:8] | vw[8:16]
    vb = pltpu.bitcast((vb | (vb << 16)) & 0x60000000, _f32)
    return jnp.concatenate(
        [jnp.sum(kf * kf, axis=0, keepdims=True),
         jnp.max(vb, axis=0, keepdims=True)], axis=0)


@jax.jit
def _weights(q, kmax):
    qs = q.astype(_f32) * (q.shape[0] ** -0.5 * _LOG2E)
    qn = jnp.sum(qs * qs, axis=0, keepdims=True)
    qn = jnp.maximum(jnp.maximum(qn[:, :_T], qn[:, _T:]), _TINY)
    b2 = jnp.maximum(qn * kmax, 2.0 ** -40)
    e2 = (pltpu.bitcast(b2, _i32) >> 23) + 1
    b = pltpu.bitcast(((e2 + 128) >> 1) << 23, _f32)
    b = jnp.where(b2 < _BMAX * _BMAX, b, jnp.nan)
    row = lax.broadcasted_iota(_i32, (16, _T), 0)
    coef = jnp.where(
        row == 0, -2.0 ** 24, jnp.where(
            row == 4, -1.5 * 2.0 ** 12, jnp.where(
                row == 8, 2.0 ** 24, jnp.where(row == 12, -1.0, 0.0))))
    return jnp.concatenate(
        [qs[:, :_T] * 2.0 ** 11, coef * b, qs[:, _T:]], axis=0).astype(_bf16)


@jax.jit
def _logits(kw, q):
    s = jnp.dot(pltpu.bitcast(kw, _bf16), q, preferred_element_type=_f32)
    return s, jnp.max(s.reshape(_T // 8, 8, _T), axis=0)


@jax.jit
def _exp_shifted(s, m):
    p = jnp.exp2((s.reshape(_T // 8, 8, _T) - m) * (32 ** -0.5 * _LOG2E))
    return p.reshape(_T, _T), jnp.sum(p, axis=0)


def _self_test():
    def keys(r, d):
        return (((r * 7 + d * 11 + (r >> 4) * d) & 15) - 8).astype(_f32) * 0.0625

    r = lax.broadcasted_iota(_i32, (_T, _KA), 0)
    c = lax.broadcasted_iota(_i32, (_T, _KA), 1)
    ka = jnp.where((c >= 32) & (c < 48), 1.0, keys(r, jnp.where(c < 32, c, c - 48)))
    d = lax.broadcasted_iota(_i32, (32, 2 * _T), 0)
    j = lax.broadcasted_iota(_i32, (32, 2 * _T), 1)
    q = (((d * 5 + j * 3 + (j >> 4) * d) & 15) - 8).astype(_f32) * 0.125
    w = _weights(q.astype(_bf16), jnp.full((1, _T), 8.5, _f32))
    p, _ = _probs(pltpu.bitcast(ka.astype(_bf16), _u32), w)
    r = lax.broadcasted_iota(_i32, (_T, 32), 0)
    k = keys(_T - 8 - (r & -8) + (r & 7), lax.broadcasted_iota(_i32, (_T, 32), 1))
    wf = w.astype(_f32)
    s = jnp.dot(k, jnp.concatenate([wf[:32] * 2.0 ** -11, wf[48:]], axis=1),
                preferred_element_type=_f32)
    ratio = p * jnp.exp2(-s)
    ok = jnp.max(ratio, axis=0, keepdims=True) < 1.02 * jnp.min(ratio, axis=0, keepdims=True)
    bad = jnp.where(ok, 0.0, jnp.nan)
    return bad[:, :_T] + bad[:, _T:]


def _kernel(q_hbm, k_hbm, v_hbm, o_hbm, q_all, k_all, v_all, o_all,
            ka_scr, vf_scr, st_scr, w_scr, fl_scr, ks_scr, vb_scr, z_scr, isem, osem):
    T, HB = _T, _HB
    BH, D, S = q_hbm.shape
    NS = (BH - 1) // HB
    NC = S // T
    NQ = S // (2 * T)

    def in_copies(g, n, slot):
        return [pltpu.make_async_copy(a.at[pl.ds(g, n)], b.at[pl.ds(g, n)], isem.at[slot])
                for a, b in ((k_hbm, k_all), (v_hbm, v_all), (q_hbm, q_all))]

    def cols_copy(src, dst, g, lo, hi, sem):
        return pltpu.make_async_copy(src.at[g, :, pl.ds(lo, hi - lo)],
                                     dst.at[g, :, pl.ds(lo, hi - lo)], sem)

    def out_copy(g, lo, hi):
        return cols_copy(o_all, o_hbm, g, lo, hi, osem.at[0])

    def max_key_norm(g):
        m = None
        for c in range(NC):
            kn = _norms(k_all[g, :, c * T:(c + 1) * T], v_all[g, :, c * T:(c + 1) * T])
            if m is not None:
                kn = jnp.maximum(kn, m)
            m = jnp.max(kn, axis=1, keepdims=True)
        mb = jnp.broadcast_to(m, (2, T))
        return jnp.where(mb[1:2] == 0.0, jnp.inf, jnp.maximum(mb[0:1], _TINY) * 1.05)

    def weights(g, i, kmax):
        return _weights(q_all[g, :, 2 * i * T:(2 * i + 2) * T], kmax)

    def stage_k(g, buf, c):
        ka_scr[buf, c * T // 2:(c + 1) * T // 2, :] = _stage_k(k_all[g, :, c * T:(c + 1) * T])

    def stage_v(g, buf, c):
        vf_scr[buf, :, c * T:(c + 1) * T] = v_all[g, :, c * T:(c + 1) * T].astype(_f32)
        vb_scr[buf, :, c * T:(c + 1) * T] = pltpu.bitcast(v_all[g, :, c * T:(c + 1) * T], _u32)

    def block(gs, bufs, lo=1, hi=None):
        first = hi is not None
        nh = 1 if first else len(gs) - 1
        units = []
        for h in range(nh):
            rest = [(h, i, c) for i in range(1, NQ) for c in range(NC)]
            n = len(rest) - _START
            pos = [] if first else [_START + (c * n) // NC for c in range(NC)]
            for j, u in enumerate(rest):
                if j in pos:
                    units.append((h + 1, 0, pos.index(j)))
                if h > 0 or lo <= u[1] < (hi or NQ):
                    units.append(u)
        accs, ls, ps, ws, chk = {}, {}, {}, {}, {}
        kmaxs = {0: st_scr[0:1, :]}
        if not first:
            ws[0, lo] = pltpu.bitcast(w_scr[...], _bf16)
        if lo > 1:
            chk[0] = st_scr[1:2, :]

        def qk(u, split):
            h, i, c = u
            g, buf = gs[h], bufs[h]
            if i == 0 and c == 0:
                kmaxs[h] = max_key_norm(g)
            if (h, i) not in ws:
                ws[h, i] = weights(g, i, kmaxs[h])
            if i == 0 or (first and i == 1):
                if i == 0 or c >= _NPRE:
                    stage_k(g, buf, c)
                stage_v(g, buf, c)
            ps[u], part = _probs(
                ka_scr[buf, c * T // 2:(c + 1) * T // 2, :], ws[h, i], split)
            ls[h, i] = part if c == 0 else ls[h, i] + part
            if i < NQ - 1 and c == _KDEP[min(i, 1)]:
                kmaxs[h] = jnp.maximum(kmaxs[h], -part[0:1, :T])
                if h == nh:
                    st_scr[0:1, :] = kmaxs[h]
                if h == nh or (first and i == hi - 1):
                    w_scr[...] = pltpu.bitcast(weights(g, i + 1, kmaxs[h]), _u32)

        def pv(u):
            h, i, c = u
            g, buf = gs[h], bufs[h]
            p = ps.pop(u)
            rs = (jnp.dot(pltpu.bitcast(vb_scr[buf, :, c * T:(c + 1) * T], _bf16),
                          p[:, :T].astype(_bf16), preferred_element_type=_f32),
                  jnp.dot(vf_scr[buf, :, c * T:(c + 1) * T], p[:, T:],
                          preferred_element_type=_f32))
            accs[h, i] = rs if c == 0 else [r + a for r, a in zip(rs, accs[h, i])]
            if c < NC - 1:
                return
            lsum = jnp.sum(ls[h, i], axis=0, keepdims=True)
            o_all[g, :, 2 * i * T:2 * (i + 1) * T] = (
                jnp.concatenate(accs[h, i], axis=1) * pl.reciprocal(lsum, approx=False)
            ).astype(o_all.dtype)
            l1 = lsum[:, :T]
            if i == 0:
                fl_scr[0, pl.ds(g, 1), :] = l1
                if h == nh:
                    out_copy(g, 0, 2 * T).start()
                return
            chk[h] = chk[h] + l1 if h in chk else l1
            olo = 2 * T if h == 0 else 0
            if first and i == hi - 1:
                st_scr[1:2, :] = chk[h]
            if i == NQ - 2 and h == nh - 1:
                out_copy(g, olo, S - 2 * T).start()
            if i == NQ - 1:
                fl_scr[1, pl.ds(g, 1), :] = chk[h]
                out_copy(g, S - 2 * T if h == nh - 1 else olo, S).start()

        done = 0
        for j in range(len(units)):
            qk(units[j], _SPLIT.get(j, 0) or _SPLIT.get(j - len(units), 0))
            while _FILL - 1 <= j < len(units) - _ENDL and done <= j - _LAG:
                pv(units[done])
                done += 1
        while done < len(units):
            pv(units[done])
            done += 1

    bufs = [h % 2 for h in range(HB)] + [0]
    if HB % 2:
        bufs[HB - 1] = 2

    qa = 2 * T * (_NA + 2)

    def first_k():
        return [cols_copy(k_hbm, k_all, 0, 0, S, isem.at[0])]

    def first_qv():
        return [cols_copy(q_hbm, q_all, 0, 2 * T, qa, isem.at[1]),
                cols_copy(v_hbm, v_all, 0, 0, S, isem.at[1])]

    def second():
        return [cols_copy(q_hbm, q_all, 0, qa, S, isem.at[3]),
                cols_copy(q_hbm, q_all, 0, 0, 2 * T, isem.at[3])] + in_copies(1, 1, 3)

    for cp in first_k() + first_qv() + second() + in_copies(2, HB, 2):
        cp.start()
    st_scr[2:3, :] = _self_test()
    z_scr[...] = jnp.zeros(z_scr.shape, _i32)
    for cp in first_k():
        cp.wait()
    kf = k_all[0].astype(_f32)
    m0 = jnp.max(jnp.sum(kf * kf, axis=0, keepdims=True), axis=1, keepdims=True)
    st_scr[0:1, :] = jnp.maximum(jnp.broadcast_to(m0, (1, T)), _TINY) * 1.05
    for c in range(_NPRE):
        stage_k(0, 1, c)
    for cp in first_qv():
        cp.wait()
    block([0], [1], 1, 1 + _NA)
    for cp in second():
        cp.wait()
    block([0, 1], [1, 0], 1 + _NA)

    def step(s, carry):
        base = 1 + s * HB

        @pl.when(s < NS - 1)
        def _():
            for cp in in_copies(base + 1, HB, 2):
                cp.wait()

        @pl.when(s == NS - 1)
        def _():
            for cp in in_copies(base + 1, HB - 1, 2):
                cp.wait()

        @pl.when(s < NS - 2)
        def _():
            for cp in in_copies(base + 1 + HB, HB, 2):
                cp.start()

        @pl.when(s == NS - 2)
        def _():
            for cp in in_copies(base + 1 + HB, HB - 1, 2):
                cp.start()

        nxt = jnp.where(s == NS - 1, 0, base + HB)
        block([base + h for h in range(HB)] + [nxt], bufs)
        return carry

    lax.fori_loop(0, NS, step, 0)

    total = jnp.sum(fl_scr[0] + fl_scr[1] + st_scr[2:3, :])
    pltpu.make_async_copy(o_all, o_hbm, osem.at[0]).wait()

    def true_max_tiles(g, t0):
        ss, ms, accs, ls, maxes, sums = {}, {}, {}, {}, [], []
        zero = z_scr[...]

        def cols(t):
            return pl.ds(pl.multiple_of((t0 + t) * T, T), T)

        def qk(t, c):
            ss[t, c], mx = _logits(ks_scr[c * T // 2:(c + 1) * T // 2, :], q_all[g, :, cols(t)])
            ms[t] = mx if c == 0 else jnp.maximum(ms[t], mx)
            maxes.append(ms[t])
            if c == NC - 1:
                ms[t] = jnp.broadcast_to(jnp.max(ms[t], axis=0, keepdims=True), (8, T))

        def pv(t, c):
            m = pltpu.bitcast(ms[t], _i32)
            for x in maxes[len(sums) + NC:len(sums) + NC + 1] + sums[-3:-2]:
                m = m | (pltpu.bitcast(x, _i32) & zero)
            p, part = _exp_shifted(ss.pop((t, c)), pltpu.bitcast(m, _f32))
            ls[t] = part if c == 0 else ls[t] + part
            sums.append(ls[t])
            r = jnp.dot(vf_scr[0, :, c * T:(c + 1) * T], p, preferred_element_type=_f32)
            accs[t] = r if c == 0 else r + accs[t]
            if c == NC - 1:
                l = jnp.sum(ls[t], axis=0, keepdims=True)
                o_all[g, :, cols(t)] = (accs[t] / l).astype(o_all.dtype)

        units = [(t, c) for t in range(_NT) for c in range(NC)]
        for j in range(len(units) + NC + _OFF):
            if j < len(units):
                qk(*units[j])
            if j >= NC + _OFF:
                pv(*units[j - NC - _OFF])

    @pl.when(jnp.logical_not(total < 1e30))
    def _():
        def head(g, carry):
            tg = jnp.sum(fl_scr[0, pl.ds(g, 1), :] + fl_scr[1, pl.ds(g, 1), :]
                         + st_scr[2:3, :])

            @pl.when(jnp.logical_not(tg < 1e30))
            def _():
                ks_scr[...] = pltpu.bitcast(k_all[g].T, _u32)
                vf_scr[0] = v_all[g].astype(_f32)

                def tiles(j, carry):
                    true_max_tiles(g, j * _NT)
                    return carry

                lax.fori_loop(0, S // (T * _NT), tiles, 0)
                cp = out_copy(g, 0, S)
                cp.start()
                cp.wait()

            return carry

        lax.fori_loop(0, BH, head, 0)


@jax.jit
def pallas_standalone__fused_io_aware_attn__prompt_kernel(
    q: jax.Array,
    k: jax.Array,
    v: jax.Array,
):
    B, H, S, D = q.shape
    BH = B * H
    assert (BH - 1) % _HB == 0 and (BH - 1) // _HB >= 2 and D == 32 and S == 2048
    qt, kt, vt = (jnp.swapaxes(x, -1, -2).reshape(BH, D, S) for x in (q, k, v))
    hbm = pl.BlockSpec(memory_space=pl.ANY)
    o = pl.pallas_call(
        _kernel,
        in_specs=[hbm, hbm, hbm],
        out_specs=hbm,
        out_shape=jax.ShapeDtypeStruct((BH, D, S), q.dtype),
        scratch_shapes=[
            pltpu.VMEM((BH, D, S), q.dtype),
            pltpu.VMEM((BH, D, S), q.dtype),
            pltpu.VMEM((BH, D, S), q.dtype),
            pltpu.VMEM((BH, D, S), q.dtype),
            pltpu.VMEM((3, S // 2, _KA), _u32),
            pltpu.VMEM((3, D, S), _f32),
            pltpu.VMEM((8, _T), _f32),
            pltpu.VMEM((_KA // 2, _T), _u32),
            pltpu.VMEM((2, BH, _T), _f32),
            pltpu.VMEM((S // 2, D), _u32),
            pltpu.VMEM((3, D // 2, S), _u32),
            pltpu.VMEM((8, _T), _i32),
            pltpu.SemaphoreType.DMA((4,)),
            pltpu.SemaphoreType.DMA((1,)),
        ],
        compiler_params=pltpu.CompilerParams(
            vmem_limit_bytes=100 * 1024 * 1024,
            disable_bounds_checks=True),
    )(qt, kt, vt)
    return jnp.swapaxes(o.reshape(B, H, D, S), -1, -2)
```

```python
import functools

import jax
import jax.numpy as jnp
from jax import lax
import jax.experimental.pallas as pl
import jax.experimental.pallas.tpu as pltpu

_LOG2E = 1.4426950408889634
_T = 128
_KA = 80
_HB = 7
_LAG = 6
_FILL = 9
_ENDL = 6
_SPLIT = {0: 112, 12: 32, -9: 80}
_START = 76
_KDEP = (6, 7)
_NA = 2
_NPRE = 6
_BMAX = 8.0
_TINY = 2.0 ** -110
_NT = 8
_OFF = 8

_f32, _bf16, _i32, _u32 = jnp.float32, jnp.bfloat16, jnp.int32, jnp.uint32


@jax.jit
def _stage_k(kc):
    ka = jnp.concatenate([kc, jnp.ones((16, _T), _bf16), kc], axis=0).T
    kw = pltpu.bitcast(ka, _u32)
    return jnp.concatenate(
        [pltpu.roll(kw[j * 8:j * 8 + 8], 4, 0) for j in reversed(range(_T // 16))],
        axis=0)


@functools.partial(jax.jit, static_argnums=2)
def _probs(kw, w, split=0):
    parts = [kw[:split // 2], kw[split // 2:]] if split else [kw]
    t = jnp.concatenate(
        [jnp.dot(pltpu.bitcast(x, _bf16), w, preferred_element_type=_f32) for x in parts],
        axis=0)
    hi = pltpu.bitcast(pltpu.bitcast(t, _i32) & (-4096), _f32)
    p = jnp.concatenate([jnp.exp2(t * 2.0 ** -11), jnp.exp2(t - hi)], axis=1)
    part = jnp.sum(p.reshape(_T // 8, 8, 2 * _T), axis=0)
    p = jnp.concatenate(
        [p[j * 8:j * 8 + 8] for j in reversed(range(_T // 8))], axis=0)
    return p, part


@jax.jit
def _pv(vw, vf, p, acc):
    rs = [jnp.dot(pltpu.bitcast(vw, _bf16), p[:, :_T].astype(_bf16),
                  preferred_element_type=_f32),
          jnp.dot(vf, p[:, _T:], preferred_element_type=_f32)]
    return rs if acc is None else [r + a for r, a in zip(rs, acc)]


@jax.jit
def _norms(kc, vc):
    kf = kc.astype(_f32)
    vw = pltpu.bitcast(vc, _i32)
    vb = vw[0:8] | vw[8:16]
    vb = pltpu.bitcast((vb | (vb << 16)) & 0x60000000, _f32)
    return jnp.concatenate(
        [jnp.sum(kf * kf, axis=0, keepdims=True),
         jnp.max(vb, axis=0, keepdims=True)], axis=0)


@jax.jit
def _weights(q, kmax):
    qs = q.astype(_f32) * (q.shape[0] ** -0.5 * _LOG2E)
    qn = jnp.sum(qs * qs, axis=0, keepdims=True)
    qn = jnp.maximum(jnp.maximum(qn[:, :_T], qn[:, _T:]), _TINY)
    b2 = jnp.maximum(qn * kmax, 2.0 ** -40)
    e2 = (pltpu.bitcast(b2, _i32) >> 23) + 1
    b = pltpu.bitcast(((e2 + 128) >> 1) << 23, _f32)
    b = jnp.where(b2 < _BMAX * _BMAX, b, jnp.nan)
    row = lax.broadcasted_iota(_i32, (16, _T), 0)
    coef = jnp.where(
        row == 0, -2.0 ** 24, jnp.where(
            row == 4, -1.5 * 2.0 ** 12, jnp.where(
                row == 8, 2.0 ** 24, jnp.where(row == 12, -1.0, 0.0))))
    return jnp.concatenate(
        [qs[:, :_T] * 2.0 ** 11, coef * b, qs[:, _T:]], axis=0).astype(_bf16)


@jax.jit
def _logits(kw, q):
    s = jnp.dot(pltpu.bitcast(kw, _bf16), q, preferred_element_type=_f32)
    return s, jnp.max(s.reshape(_T // 8, 8, _T), axis=0)


@jax.jit
def _exp_shifted(s, m):
    p = jnp.exp2((s.reshape(_T // 8, 8, _T) - m) * (32 ** -0.5 * _LOG2E))
    return p.reshape(_T, _T), jnp.sum(p, axis=0)


def _self_test():
    def keys(r, d):
        return (((r * 7 + d * 11 + (r >> 4) * d) & 15) - 8).astype(_f32) * 0.0625

    r = lax.broadcasted_iota(_i32, (_T, _KA), 0)
    c = lax.broadcasted_iota(_i32, (_T, _KA), 1)
    ka = jnp.where((c >= 32) & (c < 48), 1.0, keys(r, jnp.where(c < 32, c, c - 48)))
    d = lax.broadcasted_iota(_i32, (32, 2 * _T), 0)
    j = lax.broadcasted_iota(_i32, (32, 2 * _T), 1)
    q = (((d * 5 + j * 3 + (j >> 4) * d) & 15) - 8).astype(_f32) * 0.125
    w = _weights(q.astype(_bf16), jnp.full((1, _T), 8.5, _f32))
    p, _ = _probs(pltpu.bitcast(ka.astype(_bf16), _u32), w)
    r = lax.broadcasted_iota(_i32, (_T, 32), 0)
    k = keys(_T - 8 - (r & -8) + (r & 7), lax.broadcasted_iota(_i32, (_T, 32), 1))
    wf = w.astype(_f32)
    s = jnp.dot(k, jnp.concatenate([wf[:32] * 2.0 ** -11, wf[48:]], axis=1),
                preferred_element_type=_f32)
    ratio = p * jnp.exp2(-s)
    ok = jnp.max(ratio, axis=0, keepdims=True) < 1.02 * jnp.min(ratio, axis=0, keepdims=True)
    bad = jnp.where(ok, 0.0, jnp.nan)
    return bad[:, :_T] + bad[:, _T:]


def _kernel(q_hbm, k_hbm, v_hbm, o_hbm, q_all, k_all, v_all, o_all,
            ka_scr, vf_scr, st_scr, w_scr, fl_scr, ks_scr, vb_scr, z_scr, isem, osem):
    T, HB = _T, _HB
    BH, D, S = q_hbm.shape
    NS = (BH - 1) // HB
    NC = S // T
    NQ = S // (2 * T)

    def in_copies(g, n, slot):
        return [pltpu.make_async_copy(a.at[pl.ds(g, n)], b.at[pl.ds(g, n)], isem.at[slot])
                for a, b in ((k_hbm, k_all), (v_hbm, v_all), (q_hbm, q_all))]

    def cols_copy(src, dst, g, lo, hi, sem):
        return pltpu.make_async_copy(src.at[g, :, pl.ds(lo, hi - lo)],
                                     dst.at[g, :, pl.ds(lo, hi - lo)], sem)

    def out_copy(g, lo, hi):
        return cols_copy(o_all, o_hbm, g, lo, hi, osem.at[0])

    def max_key_norm(g):
        m = None
        for c in range(NC):
            kn = _norms(k_all[g, :, c * T:(c + 1) * T], v_all[g, :, c * T:(c + 1) * T])
            if m is not None:
                kn = jnp.maximum(kn, m)
            m = jnp.max(kn, axis=1, keepdims=True)
        mb = jnp.broadcast_to(m, (2, T))
        return jnp.where(mb[1:2] == 0.0, jnp.inf, jnp.maximum(mb[0:1], _TINY) * 1.05)

    def weights(g, i, kmax):
        return _weights(q_all[g, :, 2 * i * T:(2 * i + 2) * T], kmax)

    def stage_k(g, buf, c):
        ka_scr[buf, c * T // 2:(c + 1) * T // 2, :] = _stage_k(k_all[g, :, c * T:(c + 1) * T])

    def stage_v(g, buf, c):
        vf_scr[buf, :, c * T:(c + 1) * T] = v_all[g, :, c * T:(c + 1) * T].astype(_f32)
        vb_scr[buf, :, c * T:(c + 1) * T] = pltpu.bitcast(v_all[g, :, c * T:(c + 1) * T], _u32)

    def block(gs, bufs, lo=1, hi=None):
        first = hi is not None
        nh = 1 if first else len(gs) - 1
        units = []
        for h in range(nh):
            rest = [(h, i, c) for i in range(1, NQ) for c in range(NC)]
            n = len(rest) - _START
            pos = [] if first else [_START + (c * n) // NC for c in range(NC)]
            for j, u in enumerate(rest):
                if j in pos:
                    units.append((h + 1, 0, pos.index(j)))
                if h > 0 or lo <= u[1] < (hi or NQ):
                    units.append(u)
        accs, ls, ps, ws, chk = {}, {}, {}, {}, {}
        kmaxs = {0: st_scr[0:1, :]}
        if not first:
            ws[0, lo] = pltpu.bitcast(w_scr[...], _bf16)
        if lo > 1:
            chk[0] = st_scr[1:2, :]

        def qk(u, split):
            h, i, c = u
            g, buf = gs[h], bufs[h]
            if i == 0 and c == 0:
                kmaxs[h] = max_key_norm(g)
            if (h, i) not in ws:
                ws[h, i] = weights(g, i, kmaxs[h])
            if i == 0 or (first and i == 1):
                if i == 0 or c >= _NPRE:
                    stage_k(g, buf, c)
                stage_v(g, buf, c)
            ps[u], part = _probs(
                ka_scr[buf, c * T // 2:(c + 1) * T // 2, :], ws[h, i], split)
            ls[h, i] = part if c == 0 else ls[h, i] + part
            if i < NQ - 1 and c == _KDEP[min(i, 1)]:
                kmaxs[h] = jnp.maximum(kmaxs[h], -part[0:1, :T])
                if h == nh:
                    st_scr[0:1, :] = kmaxs[h]
                if h == nh or (first and i == hi - 1):
                    w_scr[...] = pltpu.bitcast(weights(g, i + 1, kmaxs[h]), _u32)

        def pv(u):
            h, i, c = u
            g, buf = gs[h], bufs[h]
            accs[h, i] = _pv(vb_scr[buf, :, c * T:(c + 1) * T],
                             vf_scr[buf, :, c * T:(c + 1) * T], ps.pop(u), accs.get((h, i)))
            if c < NC - 1:
                return
            lsum = jnp.sum(ls[h, i], axis=0, keepdims=True)
            o_all[g, :, 2 * i * T:2 * (i + 1) * T] = (
                jnp.concatenate(accs[h, i], axis=1) * pl.reciprocal(lsum, approx=False)
            ).astype(o_all.dtype)
            l1 = lsum[:, :T]
            if i == 0:
                fl_scr[0, pl.ds(g, 1), :] = l1
                if h == nh:
                    out_copy(g, 0, 2 * T).start()
                return
            chk[h] = chk[h] + l1 if h in chk else l1
            olo = 2 * T if h == 0 else 0
            if first and i == hi - 1:
                st_scr[1:2, :] = chk[h]
            if i == NQ - 2 and h == nh - 1:
                out_copy(g, olo, S - 2 * T).start()
            if i == NQ - 1:
                fl_scr[1, pl.ds(g, 1), :] = chk[h]
                out_copy(g, S - 2 * T if h == nh - 1 else olo, S).start()

        done = 0
        for j in range(len(units)):
            qk(units[j], _SPLIT.get(j, 0) or _SPLIT.get(j - len(units), 0))
            while _FILL - 1 <= j < len(units) - _ENDL and done <= j - _LAG:
                pv(units[done])
                done += 1
        while done < len(units):
            pv(units[done])
            done += 1

    bufs = [h % 2 for h in range(HB)] + [0]
    if HB % 2:
        bufs[HB - 1] = 2

    qa = 2 * T * (_NA + 2)

    def first_k():
        return [cols_copy(k_hbm, k_all, 0, 0, S, isem.at[0])]

    def first_qv():
        return [cols_copy(q_hbm, q_all, 0, 2 * T, qa, isem.at[1]),
                cols_copy(v_hbm, v_all, 0, 0, S, isem.at[1])]

    def second():
        return [cols_copy(q_hbm, q_all, 0, qa, S, isem.at[3]),
                cols_copy(q_hbm, q_all, 0, 0, 2 * T, isem.at[3])] + in_copies(1, 1, 3)

    for cp in first_k() + first_qv() + second() + in_copies(2, HB, 2):
        cp.start()
    st_scr[2:3, :] = _self_test()
    z_scr[...] = jnp.zeros(z_scr.shape, _i32)
    for cp in first_k():
        cp.wait()
    kf = k_all[0].astype(_f32)
    m0 = jnp.max(jnp.sum(kf * kf, axis=0, keepdims=True), axis=1, keepdims=True)
    st_scr[0:1, :] = jnp.maximum(jnp.broadcast_to(m0, (1, T)), _TINY) * 1.05
    for c in range(_NPRE):
        stage_k(0, 1, c)
    for cp in first_qv():
        cp.wait()
    block([0], [1], 1, 1 + _NA)
    for cp in second():
        cp.wait()
    block([0, 1], [1, 0], 1 + _NA)

    def step(s, carry):
        base = 1 + s * HB

        @pl.when(s < NS - 1)
        def _():
            for cp in in_copies(base + 1, HB, 2):
                cp.wait()

        @pl.when(s == NS - 1)
        def _():
            for cp in in_copies(base + 1, HB - 1, 2):
                cp.wait()

        @pl.when(s < NS - 2)
        def _():
            for cp in in_copies(base + 1 + HB, HB, 2):
                cp.start()

        @pl.when(s == NS - 2)
        def _():
            for cp in in_copies(base + 1 + HB, HB - 1, 2):
                cp.start()

        nxt = jnp.where(s == NS - 1, 0, base + HB)
        block([base + h for h in range(HB)] + [nxt], bufs)
        return carry

    lax.fori_loop(0, NS, step, 0)

    total = jnp.sum(fl_scr[0] + fl_scr[1] + st_scr[2:3, :])
    pltpu.make_async_copy(o_all, o_hbm, osem.at[0]).wait()

    def true_max_tiles(g, t0):
        ss, ms, accs, ls, maxes, sums = {}, {}, {}, {}, [], []
        zero = z_scr[...]

        def cols(t):
            return pl.ds(pl.multiple_of((t0 + t) * T, T), T)

        def qk(t, c):
            ss[t, c], mx = _logits(ks_scr[c * T // 2:(c + 1) * T // 2, :], q_all[g, :, cols(t)])
            ms[t] = mx if c == 0 else jnp.maximum(ms[t], mx)
            maxes.append(ms[t])
            if c == NC - 1:
                ms[t] = jnp.broadcast_to(jnp.max(ms[t], axis=0, keepdims=True), (8, T))

        def pv(t, c):
            m = pltpu.bitcast(ms[t], _i32)
            for x in maxes[len(sums) + NC:len(sums) + NC + 1] + sums[-3:-2]:
                m = m | (pltpu.bitcast(x, _i32) & zero)
            p, part = _exp_shifted(ss.pop((t, c)), pltpu.bitcast(m, _f32))
            ls[t] = part if c == 0 else ls[t] + part
            sums.append(ls[t])
            r = jnp.dot(vf_scr[0, :, c * T:(c + 1) * T], p, preferred_element_type=_f32)
            accs[t] = r if c == 0 else r + accs[t]
            if c == NC - 1:
                l = jnp.sum(ls[t], axis=0, keepdims=True)
                o_all[g, :, cols(t)] = (accs[t] / l).astype(o_all.dtype)

        units = [(t, c) for t in range(_NT) for c in range(NC)]
        for j in range(len(units) + NC + _OFF):
            if j < len(units):
                qk(*units[j])
            if j >= NC + _OFF:
                pv(*units[j - NC - _OFF])

    @pl.when(jnp.logical_not(total < 1e30))
    def _():
        def head(g, carry):
            tg = jnp.sum(fl_scr[0, pl.ds(g, 1), :] + fl_scr[1, pl.ds(g, 1), :]
                         + st_scr[2:3, :])

            @pl.when(jnp.logical_not(tg < 1e30))
            def _():
                ks_scr[...] = pltpu.bitcast(k_all[g].T, _u32)
                vf_scr[0] = v_all[g].astype(_f32)

                def tiles(j, carry):
                    true_max_tiles(g, j * _NT)
                    return carry

                lax.fori_loop(0, S // (T * _NT), tiles, 0)
                cp = out_copy(g, 0, S)
                cp.start()
                cp.wait()

            return carry

        lax.fori_loop(0, BH, head, 0)


@jax.jit
def pallas_standalone__fused_io_aware_attn__prompt_kernel(
    q: jax.Array,
    k: jax.Array,
    v: jax.Array,
):
    B, H, S, D = q.shape
    BH = B * H
    assert (BH - 1) % _HB == 0 and (BH - 1) // _HB >= 2 and D == 32 and S == 2048
    qt, kt, vt = (jnp.swapaxes(x, -1, -2).reshape(BH, D, S) for x in (q, k, v))
    hbm = pl.BlockSpec(memory_space=pl.ANY)
    o = pl.pallas_call(
        _kernel,
        in_specs=[hbm, hbm, hbm],
        out_specs=hbm,
        out_shape=jax.ShapeDtypeStruct((BH, D, S), q.dtype),
        scratch_shapes=[
            pltpu.VMEM((BH, D, S), q.dtype),
            pltpu.VMEM((BH, D, S), q.dtype),
            pltpu.VMEM((BH, D, S), q.dtype),
            pltpu.VMEM((BH, D, S), q.dtype),
            pltpu.VMEM((3, S // 2, _KA), _u32),
            pltpu.VMEM((3, D, S), _f32),
            pltpu.VMEM((8, _T), _f32),
            pltpu.VMEM((_KA // 2, _T), _u32),
            pltpu.VMEM((2, BH, _T), _f32),
            pltpu.VMEM((S // 2, D), _u32),
            pltpu.VMEM((3, D // 2, S), _u32),
            pltpu.VMEM((8, _T), _i32),
            pltpu.SemaphoreType.DMA((4,)),
            pltpu.SemaphoreType.DMA((1,)),
        ],
        compiler_params=pltpu.CompilerParams(
            vmem_limit_bytes=100 * 1024 * 1024,
            disable_bounds_checks=True),
    )(qt, kt, vt)
    return jnp.swapaxes(o.reshape(B, H, D, S), -1, -2)
```
